```python
import jax
import jax.numpy as jnp

def _softmax(x, axis=-1):
    return jax.nn.softmax(x, axis=axis)
def _gelu(x):
    return jax.nn.gelu(x, approximate=True)
def _silu(x):
    return jax.nn.silu(x)
def _sigmoid(x):
    return jax.nn.sigmoid(x)
def _layernorm(x, axis=-1, eps=1e-5):
    m = jnp.mean(x, axis=axis, keepdims=True)
    v = jnp.var(x, axis=axis, keepdims=True)
    return (x - m) / jnp.sqrt(v + eps)
def _scatter_add(tgt, idx, src, axis=0):
    return tgt.at[idx].add(src)
def _segment_sum(src, seg, n):
    return jax.ops.segment_sum(src, seg, n)
class _Rng:
    def __init__(self, key):
        self._k = key
    def _next(self):
        self._k, sub = jax.random.split(self._k)
        return sub
    def normal(self, shape):
        return jax.random.normal(self._next(), shape, dtype=jnp.bfloat16)
    def randint(self, lo, hi, shape):
        return jax.random.randint(self._next(), shape, lo, hi, dtype=jnp.int32)
    def uniform(self, shape, lo=0.0, hi=1.0):
        return jax.random.uniform(self._next(), shape, jnp.bfloat16, lo, hi)
    def permutation(self, n):
        return jax.random.permutation(self._next(), n)


kernel_name = 'concat_heads__mha_block_cached__compressed_kv_cla__decode'

def setup_inputs():
    _rng = _Rng(jax.random.key(int.from_bytes(__import__("os").urandom(4), "little")))
    _w = (lambda a: (lambda t: t.astype(jnp.bfloat16) if jnp.issubdtype(t.dtype, jnp.floating) else t)(jnp.asarray(a)))
    def _A_setup():
        B, Sq, D = 4, 1, 576
        H, Sk, Dh = 32, 4096, 128
        return {
            "x": _w((lambda *s: _rng.normal(s) * 0.05)(B, Sq, D)),
            "k_cache": _w((lambda *s: _rng.normal(s) * 0.05)(B, H, Sk, Dh)),
            "v_cache": _w((lambda *s: _rng.normal(s) * 0.05)(B, H, Sk, Dh)),
            "wq": _w((lambda *s: _rng.normal(s) * 0.05)(D, H * Dh) * (D ** -0.5)),
            "wo": _w((lambda *s: _rng.normal(s) * 0.05)(H * Dh, D) * ((H * Dh) ** -0.5)),
        }
    _A_in = _A_setup()

    def _B_setup():
        B, H, Sq, Sk, D, M = 4, 32, 1, 4096, 128, 576
        Dc = 4 * D
        return {
            "x": _w((lambda *s: _rng.normal(s) * 0.05)(B, Sq, M)),
            "c_kv": _w((lambda *s: _rng.normal(s) * 0.05)(B, Sk, Dc)),
            "w_q": _w((lambda *s: _rng.normal(s) * 0.05)(M, H, D) * (M ** -0.5)),
            "w_uk": _w((lambda *s: _rng.normal(s) * 0.05)(Dc, H, D) * (Dc ** -0.5)),
            "w_uv": _w((lambda *s: _rng.normal(s) * 0.05)(Dc, H, D) * (Dc ** -0.5)),
            "w_o": _w((lambda *s: _rng.normal(s) * 0.05)(H, D, M) * ((H * D) ** -0.5)),
        }
    _B_in = _B_setup()

    return {
        "A_x": _A_in["x"],
        "A_k_cache": _A_in["k_cache"],
        "A_v_cache": _A_in["v_cache"],
        "A_wq": _A_in["wq"],
        "A_wo": _A_in["wo"],
        "B_x": _B_in["x"],
        "B_c_kv": _B_in["c_kv"],
        "B_w_q": _B_in["w_q"],
        "B_w_uk": _B_in["w_uk"],
        "B_w_uv": _B_in["w_uv"],
        "B_w_o": _B_in["w_o"],
    }

def reference(A_x, A_k_cache, A_v_cache, A_wq, A_wo, B_x, B_c_kv, B_w_q, B_w_uk, B_w_uv, B_w_o):
    def _A_ref(x, k_cache, v_cache, wq, wo):
        B, Sq, D = x.shape
        H, Dh = 32, 128
        q = (lambda x, *d: x.transpose(*d))((x @ wq).reshape(B, Sq, H, Dh), 0, 2, 1, 3)
        scores = jnp.einsum("bhqd,bhkd->bhqk", q, k_cache) * (Dh ** -0.5)
        p = _softmax(scores, axis=-1)
        o = jnp.einsum("bhqk,bhkd->bhqd", p, v_cache)
        return (lambda x, *d: x.transpose(*d))(o, 0, 2, 1, 3).reshape(B, Sq, H * Dh) @ wo

    def _B_ref(x, c_kv, w_q, w_uk, w_uv, w_o):
        B, Sq, M = x.shape[0], x.shape[1], x.shape[2]
        Sk = c_kv.shape[1]
        H, D = w_q.shape[1], w_q.shape[2]
        q = jnp.einsum("bqm,mhd->bhqd", x, w_q)
        k = jnp.einsum("bkc,chd->bhkd", c_kv, w_uk)
        v = jnp.einsum("bkc,chd->bhkd", c_kv, w_uv)
        scores = jnp.einsum("bhqd,bhkd->bhqk", q, k) * (D ** -0.5)
        off = Sk - Sq
        qi = jnp.arange(Sq)[:, None]
        kj = jnp.arange(Sk)[None, :]
        cmask = kj <= (qi + off)
        scores = jnp.where(cmask[None, None], scores, -1e9)
        p = _softmax(scores, axis=-1)
        ctx = jnp.einsum("bhqk,bhkd->bhqd", p, v)
        return jnp.einsum("bhqd,hdm->bqm", ctx, w_o)

    a = _A_ref(A_x, A_k_cache, A_v_cache, A_wq, A_wo)
    b = _B_ref(B_x, B_c_kv, B_w_q, B_w_uk, B_w_uv, B_w_o)
    return jnp.concatenate([a, b], axis=-1)
```

```python
import jax
import jax.numpy as jnp
from jax import lax
import jax.experimental.pallas as pl
import jax.experimental.pallas.tpu as pltpu

_BF = jnp.bfloat16
_F32 = jnp.float32
_NT = (((1,), (1,)), ((), ()))
_NN = (((1,), (0,)), ((), ()))

_B = 4
_H = 32
_S = 4096
_D = 128
_M = 576
_C = 512
_R = 8

_NBUF = 3
_PIECE = 128
_CK = 512
_CW = 64


def _dot(a, b, dims):
    return lax.dot_general(a, b, dims, preferred_element_type=_F32)


def _kernel(xa_h, k_h, v_h, wqa_h, woa_h, xb_h, ckv_h, wqb_h, wuk_h, wuv_h, wob_h,
            out_ref,
            xa_v, xb_v, k_v, v_v, wqa_v, woa_v, ckv_v, wb_v, wob_v,
            word_s, wh_s, qa_s, oa_s, qh_s, qc_s, m_s, l_s, acc_s, cc_s, ch_s, ctx_s,
            kv_sem, w_sem):
    scale = _D ** -0.5
    n_heads = _B * _H
    SEM_XA, SEM_XB, SEM_WQA, SEM_WQB, SEM_WUK, SEM_CKV, SEM_WUV, SEM_WOA, SEM_WOB = range(9)

    def copy(src, dst, sem, prio):
        pltpu.make_async_copy(src, dst, sem).start(priority=prio)

    def wait_all(buf, sem):
        pltpu.make_async_copy(buf, buf, sem).wait()

    def rows(src, dst, sem, start, size, prio):
        copy(src.at[pl.ds(start, size)], dst.at[pl.ds(start, size)], sem, prio)

    def issue_kv(i, slot):
        for s in range(_S // _PIECE):
            sl = pl.ds(s * _PIECE, _PIECE)
            copy(k_h.at[i, sl], k_v.at[slot, sl], kv_sem.at[0, slot], 0)
            copy(v_h.at[i, sl], v_v.at[slot, sl], kv_sem.at[1, slot], 1)

    def issue_wide(src, dst, sem, t):
        r0 = pl.multiple_of(t * 16, 16)
        r1 = pl.multiple_of(t * 16 + _M // 2, 16)
        for c in range(4):
            cs = pl.ds(c * 1024, 1024)
            copy(src.at[pl.ds(r0, 16), cs], dst.at[pl.ds(r0, 16), cs], sem, 0)
            copy(src.at[pl.ds(r1, 16), cs], dst.at[pl.ds(r1, 16), cs], sem, 1)

    def pad_rows(x):
        x = x.astype(_F32)
        return jnp.concatenate([x, jnp.zeros_like(x)], axis=0).astype(_BF)

    wqb_v = wb_v.at[pl.ds(0, _M * _H)]
    wuk_v = wb_v.at[pl.ds(_M * _H, _C * _H)]
    wuv_v = wb_v.at[pl.ds((_M + _C) * _H, _C * _H)]

    def b_split_heads(t):
        n = _CW * _H
        word_s[...] = pltpu.bitcast(wb_v[pl.ds(pl.multiple_of(t * n, n), n), :], jnp.uint32)
        cs = pl.ds(pl.multiple_of(t * _CW, _CW), _CW)
        for j in range(_H // 2):
            u = word_s[pl.ds(j, _CW, stride=_H // 2), :]
            wh_s[2 * j, cs, :] = pltpu.bitcast(u << 16, _F32).astype(_BF)
            wh_s[2 * j + 1, cs, :] = pltpu.bitcast(u & jnp.uint32(0xFFFF0000), _F32).astype(_BF)

    def a_step(i, slot):
        b = i // _H
        h = i % _H
        wait_all(k_v.at[slot], kv_sem.at[0, slot])
        wait_all(v_v.at[slot], kv_sem.at[1, slot])
        s = _dot(qa_s[h].astype(_BF), k_v[slot], _NT) * scale
        m = jnp.max(s, axis=1, keepdims=True)
        p = jnp.exp(s - m)
        l = jnp.sum(p, axis=1, keepdims=True)
        o = _dot(p.astype(_BF), v_v[slot], _NN) / l
        row = lax.broadcasted_iota(jnp.int32, (_R, _D), 0)
        oa_s[h] = jnp.where(row == b, o, oa_s[h])

    def b_query(j):
        x = pad_rows(xb_v[...])
        for e in range(2):
            h = 2 * j + e
            q = _dot(x, wh_s[h, pl.ds(0, _M), :], _NN).astype(_BF)
            qh_s[pl.ds(pl.multiple_of(h * _R, _R), _R), :] = _dot(q, wh_s[h, pl.ds(_M, _C), :], _NT)

    def b_regroup_query():
        r = lax.broadcasted_iota(jnp.int32, (n_heads, _H * _R), 0)
        c = lax.broadcasted_iota(jnp.int32, (n_heads, _H * _R), 1)
        sel = jnp.where(c == (r % _H) * _R + r // _H, 1.0, 0.0).astype(_BF)
        qc_s[...] = _dot(sel, qh_s[...].astype(_BF), _NN).astype(_BF)

    def b_attend(t):
        per = _S // _CK
        b = t // per
        hs = pl.ds(pl.multiple_of(b * _H, _H), _H)

        @pl.when(t % per == 0)
        def _():
            m_s[...] = jnp.full(m_s.shape, -jnp.inf, _F32)
            l_s[...] = jnp.zeros(l_s.shape, _F32)
            acc_s[...] = jnp.zeros(acc_s.shape, _F32)

        c = ckv_v[pl.ds(pl.multiple_of(t * _CK, _CK), _CK), :]
        s = _dot(qc_s[hs, :], c, _NT) * scale
        m_old = m_s[...]
        m_new = jnp.maximum(m_old, jnp.max(s, axis=1, keepdims=True))
        alpha = jnp.exp(m_old - m_new)
        p = jnp.exp(s - m_new[:, :1])
        l_new = alpha * l_s[...] + jnp.sum(p, axis=1, keepdims=True)
        acc = alpha[:, :1] * acc_s[...] + _dot(p.astype(_BF), c, _NN)
        m_s[...] = m_new
        l_s[...] = l_new
        acc_s[...] = acc

        @pl.when(t % per == per - 1)
        def _():
            cc_s[hs, :] = (acc / l_new[:, :1]).astype(_BF)

    def b_regroup_ctx():
        r = lax.broadcasted_iota(jnp.int32, (_H * _R, n_heads), 0)
        c = lax.broadcasted_iota(jnp.int32, (_H * _R, n_heads), 1)
        sel = jnp.where(r == (c % _H) * _R + c // _H, 1.0, 0.0).astype(_BF)
        ch_s[...] = _dot(sel, cc_s[...], _NN)

    def b_value(j):
        for e in range(4):
            h = 4 * j + e
            ch = ch_s[pl.ds(pl.multiple_of(h * _R, _R), _R), :].astype(_BF)
            ctx_s[h] = _dot(ch, wh_s[h, pl.ds(_M + _C, _C), :], _NN)

    copy(xa_h, xa_v, w_sem.at[SEM_XA], 0)

    @pl.loop(0, _M // 32)
    def _(t):
        issue_wide(wqa_h, wqa_v, w_sem.at[SEM_WQA], t)

    copy(xb_h, xb_v, w_sem.at[SEM_XB], 0)
    oa_s[...] = jnp.zeros(oa_s.shape, _F32)

    @pl.loop(0, _NBUF)
    def _(i):
        issue_kv(i, i)

        @pl.when(i == 1)
        def _():
            wait_all(xa_v, w_sem.at[SEM_XA])
            wait_all(xb_v, w_sem.at[SEM_XB])
            wait_all(wqa_v, w_sem.at[SEM_WQA])

        @pl.when(jnp.logical_and(i >= 1, i < 3))
        def _():
            half = _H // 2
            c0 = pl.multiple_of((i - 1) * half * _D, half * _D)
            q = _dot(pad_rows(xa_v[...]), wqa_v[:, pl.ds(c0, half * _D)], _NN)
            for h in range(half):
                qa_s[(i - 1) * half + h] = q[:, h * _D:(h + 1) * _D]

    T_WQ, T_WUV, T_CKV = 0, 16, 24
    T_SPLIT, T_Q, T_ATT, T_VAL = 27, 52, 70, 104

    def window(i, start, n):
        return jnp.logical_and(i >= start, i < start + n)

    @pl.loop(0, n_heads - _NBUF)
    def _(i):
        slot = i % _NBUF
        a_step(i, slot)
        issue_kv(i + _NBUF, slot)

        @pl.when(window(i, T_WQ, 16))
        def _():
            nq = _M * _H // 128
            for s in range(8):
                t = (i - T_WQ) * 8 + s
                rows(wqb_h, wqb_v, w_sem.at[SEM_WQB], pl.multiple_of(t * nq, 16), nq, 0)
                rows(wuk_h, wuk_v, w_sem.at[SEM_WUK], pl.multiple_of(t * _PIECE, _PIECE), _PIECE, 1)

        @pl.when(window(i, T_CKV, 32))
        def _():
            for s in range(8):
                t = (i - T_CKV) * 8 + s
                rows(ckv_h, ckv_v, w_sem.at[SEM_CKV], pl.multiple_of(t * 32, 32), 32, 0)
                rows(ckv_h, ckv_v, w_sem.at[SEM_CKV],
                     pl.multiple_of(t * 32 + _B * _S // 2, 32), 32, 1)

        @pl.when(window(i, T_WUV, 8))
        def _():
            for s in range(8):
                t = (i - T_WUV) * 8 + s
                rows(wuv_h, wuv_v, w_sem.at[SEM_WUV], pl.multiple_of(t * _PIECE, _PIECE), _PIECE, 0)
                rows(wuv_h, wuv_v, w_sem.at[SEM_WUV],
                     pl.multiple_of(t * _PIECE + _C * _H // 2, _PIECE), _PIECE, 1)

        @pl.when(i == T_SPLIT)
        def _():
            wait_all(wqb_v, w_sem.at[SEM_WQB])
            wait_all(wuk_v, w_sem.at[SEM_WUK])
            wait_all(wuv_v, w_sem.at[SEM_WUV])

        @pl.when(window(i, T_SPLIT, (_M + 2 * _C) // _CW))
        def _():
            b_split_heads(i - T_SPLIT)

        @pl.when(window(i, T_Q, _H // 2))
        def _():
            b_query(i - T_Q)

        @pl.when(i == T_ATT - 1)
        def _():
            b_regroup_query()
            wait_all(ckv_v, w_sem.at[SEM_CKV])

        @pl.when(window(i, T_ATT, _B * _S // _CK))
        def _():
            b_attend(i - T_ATT)

        @pl.when(i == T_VAL - 1)
        def _():
            b_regroup_ctx()

        @pl.when(window(i, T_VAL, _H // 4))
        def _():
            b_value(i - T_VAL)

    @pl.loop(0, _NBUF)
    def _(t):
        i = n_heads - _NBUF + t
        a_step(i, i % _NBUF)
        per = _M // 32 // _NBUF
        for s in range(per):
            issue_wide(woa_h, woa_v, w_sem.at[SEM_WOA], t * per + s)

    @pl.loop(0, _M * _H // 2 // _PIECE)
    def _(t):
        rows(wob_h, wob_v, w_sem.at[SEM_WOB], pl.multiple_of(t * _PIECE, _PIECE), _PIECE, 0)
        rows(wob_h, wob_v, w_sem.at[SEM_WOB],
             pl.multiple_of(t * _PIECE + _M * _H // 2, _PIECE), _PIECE, 1)

    wait_all(woa_v, w_sem.at[SEM_WOA])
    oa = jnp.concatenate([oa_s[h] for h in range(_H)], axis=1).astype(_BF)
    out_a = _dot(oa, woa_v[...], _NT)

    wait_all(wob_v, w_sem.at[SEM_WOB])
    out_b = jnp.zeros((_R, _M), _F32)
    for h in range(_H):
        out_b = out_b + _dot(ctx_s[h].astype(_BF), wob_v[pl.ds(h * _M, _M), :], _NT)

    out = jnp.concatenate([out_a, out_b], axis=1)
    out_ref[...] = out[:_B].astype(out_ref.dtype)


@jax.jit
def pallas_concat_heads__mha_block_cached__compressed_kv_cla__decode_kernel(
    A_x: jax.Array,
    A_k_cache: jax.Array,
    A_v_cache: jax.Array,
    A_wq: jax.Array,
    A_wo: jax.Array,
    B_x: jax.Array,
    B_c_kv: jax.Array,
    B_w_q: jax.Array,
    B_w_uk: jax.Array,
    B_w_uv: jax.Array,
    B_w_o: jax.Array,
):
    assert A_k_cache.shape == (_B, _H, _S, _D) and B_c_kv.shape == (_B, _S, _C)
    assert A_x.shape == (_B, 1, _M) and B_x.shape == (_B, 1, _M)

    operands = (
        A_x.reshape(_B, _M),
        A_k_cache.reshape(_B * _H, _S, _D),
        A_v_cache.reshape(_B * _H, _S, _D),
        A_wq,
        A_wo.T,
        B_x.reshape(_B, _M),
        B_c_kv.reshape(_B * _S, _C),
        B_w_q.reshape(_M * _H, _D),
        B_w_uk.reshape(_C * _H, _D),
        B_w_uv.reshape(_C * _H, _D),
        B_w_o.transpose(0, 2, 1).reshape(_H * _M, _D),
    )
    out = pl.pallas_call(
        _kernel,
        out_shape=jax.ShapeDtypeStruct((_B, 2 * _M), A_x.dtype),
        in_specs=[pl.BlockSpec(memory_space=pltpu.HBM)] * len(operands),
        scratch_shapes=[
            pltpu.VMEM((_B, _M), _BF),
            pltpu.VMEM((_B, _M), _BF),
            pltpu.VMEM((_NBUF, _S, _D), _BF),
            pltpu.VMEM((_NBUF, _S, _D), _BF),
            pltpu.VMEM((_M, _H * _D), _BF),
            pltpu.VMEM((_M, _H * _D), _BF),
            pltpu.VMEM((_B * _S, _C), _BF),
            pltpu.VMEM(((_M + 2 * _C) * _H, _D), _BF),
            pltpu.VMEM((_H * _M, _D), _BF),
            pltpu.VMEM((_CW * _H // 2, _D), jnp.uint32),
            pltpu.VMEM((_H, _M + 2 * _C, _D), _BF),
            pltpu.VMEM((_H, _R, _D), _F32),
            pltpu.VMEM((_H, _R, _D), _F32),
            pltpu.VMEM((_H * _R, _C), _F32),
            pltpu.VMEM((_B * _H, _C), _BF),
            pltpu.VMEM((_H, _D), _F32),
            pltpu.VMEM((_H, _D), _F32),
            pltpu.VMEM((_H, _C), _F32),
            pltpu.VMEM((_B * _H, _C), _BF),
            pltpu.VMEM((_H * _R, _C), _F32),
            pltpu.VMEM((_H, _R, _D), _F32),
            pltpu.SemaphoreType.DMA((2, _NBUF)),
            pltpu.SemaphoreType.DMA((9,)),
        ],
        compiler_params=pltpu.CompilerParams(vmem_limit_bytes=100 * 1024 * 1024),
    )(*operands)
    return out.reshape(_B, 1, 2 * _M)
```

```python
import jax
import jax.numpy as jnp
from jax import lax
import jax.experimental.pallas as pl
import jax.experimental.pallas.tpu as pltpu

_BF = jnp.bfloat16
_F32 = jnp.float32
_NT = (((1,), (1,)), ((), ()))
_NN = (((1,), (0,)), ((), ()))

_B = 4
_H = 32
_S = 4096
_D = 128
_M = 576
_C = 512
_R = 8

_G = 8
_TK = 512
_NBUF = 4
_SEG = 64
_NW = 4
_NC = 16
_CW = 16


def _dot(a, b, dims):
    return lax.dot_general(a, b, dims, preferred_element_type=_F32)


def _tile(start, size):
    return pl.ds(pl.multiple_of(start * size, size), size)


def _kernel(xa_h, k_h, v_h, wqa_h, woa_h, xb_h, ckv_h, wqb_h, wuk_h, wuv_h, wob_h,
            out_ref,
            xa_v, xb_v, k_v, v_v, wqa_v, woa_v, ckv_v, wqb_v, wuk_v, wuv_v, wob_v,
            word_s, wqh_s, wkh_s, wvh_s,
            qah_s, qa_s, ma_s, la_s, acca_s, oa_s,
            qh_s, qc_s, mb_s, lb_s, accb_s, cc_s, ch_s, ctx_s,
            kv_sem, w_sem, wob_sem):
    scale = _D ** -0.5
    per_group = _S // _TK
    n_steps = _B * _H // _G * per_group
    XA, XB, WQA, WQB, WUK, WUV, CKV, WOA = range(8)

    def copy(src, dst, sem, prio):
        pltpu.make_async_copy(src, dst, sem).start(priority=prio)

    def wait_all(buf, sem):
        pltpu.make_async_copy(buf, buf, sem).wait()

    def fetch(src, dst, sem, pair, t, prio):
        cols = src.shape[2]
        if cols <= _C:
            idx = (pl.ds(2 * pair, 2), _tile(t, _SEG * _D // cols))
        else:
            per_row = cols * 8 // (_SEG * _D)
            idx = (pl.ds(2 * pair, 2), _tile(t // per_row, 8), _tile(t % per_row, cols // per_row))
        copy(src.at[idx], dst.at[idx], sem, prio)

    def fetch_kv(i):
        slot = i % _NBUF
        head0 = i // per_group * _G
        seg0 = i % per_group * (_TK // _SEG)

        @pl.loop(0, _TK // _SEG)
        def _(t):
            for p in range(_G // 2):
                src = (pl.ds(head0 + 2 * p, 2), _tile(seg0 + t, _SEG))
                dst = (slot, pl.ds(2 * p, 2), _tile(t, _SEG))
                copy(k_h.at[src], k_v.at[dst], kv_sem.at[0, slot], 0)
                copy(v_h.at[src], v_v.at[dst], kv_sem.at[1, slot], 1)

    def fetch_wob(u):
        per_head = _M // _SEG

        @pl.loop(0, per_head)
        def _(t):
            for p in range(2):
                fetch(wob_h, wob_v, wob_sem.at[p, u], p, u * per_head + t, p)

    def pad_rows(x):
        x = x.astype(_F32)
        return jnp.concatenate([x, jnp.zeros_like(x)], axis=0)

    def a_query(u):
        w = wqa_v[:, :, _tile(u, _G * _D)].reshape(_M, _G * _D)
        q = _dot(pad_rows(xa_v[...]).astype(_BF), w, _NN)
        for h in range(_G):
            qah_s[_tile(u * _G + h, _R), :] = q[:, h * _D:(h + 1) * _D]

    def a_regroup_query():
        for b in range(_B):
            qa_s[pl.ds(b * _H, _H), :] = qah_s[pl.ds(b, _H, stride=_R), :]

    def a_attend(i):
        slot = i % _NBUF
        hs = _tile(i // per_group, _G)

        @pl.when(i % per_group == 0)
        def _():
            ma_s[...] = jnp.full(ma_s.shape, -jnp.inf, _F32)
            la_s[...] = jnp.zeros(la_s.shape, _F32)
            acca_s[...] = jnp.zeros(acca_s.shape, _F32)

        wait_all(k_v.at[slot], kv_sem.at[0, slot])
        wait_all(v_v.at[slot], kv_sem.at[1, slot])

        def own_rows(lhs, rhs_ref, dims):
            res = _dot(lhs, rhs_ref[slot, 0], dims)
            row = lax.broadcasted_iota(jnp.int32, res.shape, 0)
            for h in range(1, _G):
                res = jnp.where(row == h, _dot(lhs, rhs_ref[slot, h], dims), res)
            return res

        s = own_rows(qa_s[hs, :].astype(_BF), k_v, _NT) * scale
        m_old = ma_s[...]
        m_new = jnp.maximum(m_old, jnp.max(s, axis=1, keepdims=True))
        alpha = jnp.exp(m_old - m_new)
        p = jnp.exp(s - m_new[:, :1])
        l_new = alpha * la_s[...] + jnp.sum(p, axis=1, keepdims=True)
        acc = alpha * acca_s[...] + own_rows(p.astype(_BF), v_v, _NN)
        ma_s[...] = m_new
        la_s[...] = l_new
        acca_s[...] = acc
        oa_s[hs, :] = acc / l_new

    def a_regroup_out():
        for h in range(_H):
            qah_s[pl.ds(h * _R, _R), :] = pad_rows(oa_s[pl.ds(h, _B, stride=_H), :])

    def a_project(u):
        o = jnp.concatenate([qah_s[_tile(u * _G + h, _R), :] for h in range(_G)], axis=1)
        w = woa_v[:, :, _tile(u, _G * _D)].reshape(_M, _G * _D)
        return _dot(o.astype(_BF), w, _NT)

    def b_split_heads(w_v, wh_s, t):
        per_range = w_v.shape[1] // (_CW * _H)

        @pl.loop(0, _NW)
        def _(r):
            word_s[...] = pltpu.bitcast(w_v[r, _tile(t, _CW * _H), :], jnp.uint32)
            cs = _tile(r * per_range + t, _CW)
            for j in range(_H // 2):
                u = word_s[pl.ds(j, _CW, stride=_H // 2), :]
                wh_s[2 * j, cs, :] = pltpu.bitcast(u << 16, _F32).astype(_BF)
                wh_s[2 * j + 1, cs, :] = pltpu.bitcast(
                    u & jnp.uint32(0xFFFF0000), _F32).astype(_BF)

    def b_query(h):
        q = _dot(pad_rows(xb_v[...]).astype(_BF), wqh_s[h], _NN)
        q = _dot(q.astype(_BF), wkh_s[h], _NT)
        for c in range(_C // _D):
            qh_s[c, _tile(h, _R), :] = q[:, c * _D:(c + 1) * _D]

    def b_regroup_query():
        for b in range(_B):
            for c in range(_C // _D):
                qc_s[pl.ds(b * _H, _H), pl.ds(c * _D, _D)] = (
                    qh_s[c, pl.ds(b, _H, stride=_R), :].astype(_BF))

    def b_attend(t):
        hs = _tile(t // per_group, _H)
        per_range = ckv_v.shape[1] // _TK

        @pl.when(t % per_group == 0)
        def _():
            mb_s[...] = jnp.full(mb_s.shape, -jnp.inf, _F32)
            lb_s[...] = jnp.zeros(lb_s.shape, _F32)
            accb_s[...] = jnp.zeros(accb_s.shape, _F32)

        lat = ckv_v[t // per_range, _tile(t % per_range, _TK), :]
        s = _dot(qc_s[hs, :], lat, _NT) * scale
        m_old = mb_s[...]
        m_new = jnp.maximum(m_old, jnp.max(s, axis=1, keepdims=True))
        alpha = jnp.exp(m_old - m_new)
        p = jnp.exp(s - m_new[:, :1])
        l_new = alpha * lb_s[...] + jnp.sum(p, axis=1, keepdims=True)
        acc = alpha[:, :1] * accb_s[...] + _dot(p.astype(_BF), lat, _NN)
        mb_s[...] = m_new
        lb_s[...] = l_new
        accb_s[...] = acc
        for c in range(_C // _D):
            cc_s[c, hs, :] = acc[:, c * _D:(c + 1) * _D] / l_new

    def b_regroup_ctx():
        @pl.loop(0, _C // _D)
        def _(c):
            for h in range(_H):
                ch_s[c, pl.ds(h * _R, _R), :] = pad_rows(cc_s[c, pl.ds(h, _B, stride=_H), :])

    def b_value(h):
        lat = jnp.concatenate([ch_s[c, _tile(h, _R), :] for c in range(_C // _D)], axis=1)
        ctx_s[h] = _dot(lat.astype(_BF), wvh_s[h], _NN)

    def b_project(p, u):
        rows = _tile(u, _M)
        wait_all(wob_v.at[pl.ds(2 * p, 2), rows], wob_sem.at[p, u])
        parts = [_dot(ctx_s[r * (_H // _NW) + u].astype(_BF), wob_v[r, rows, :], _NT)
                 for r in (2 * p, 2 * p + 1)]
        return parts[0] + parts[1]

    n_wide = _M * _H // _NW // _SEG
    n_narrow = _C * _H // _NW // _SEG

    @pl.loop(0, n_wide)
    def _(t):
        for p in range(_NW // 2):
            fetch(wqa_h, wqa_v, w_sem.at[WQA], p, t, 0)
            fetch(wqb_h, wqb_v, w_sem.at[WQB], p, t, 1)

        @pl.when(t < n_narrow)
        def _():
            for p in range(_NW // 2):
                fetch(wuk_h, wuk_v, w_sem.at[WUK], p, t, 0)
                fetch(wuv_h, wuv_v, w_sem.at[WUV], p, t, 1)

        for p in range(_NW // 2):
            fetch(woa_h, woa_v, w_sem.at[WOA], p, t, p)

    copy(xa_h, xa_v, w_sem.at[XA], 0)
    copy(xb_h, xb_v, w_sem.at[XB], 1)

    @pl.loop(0, 8)
    def _(u):
        @pl.loop(0, 8)
        def _(t):
            for p in range(_NC // 4):
                fetch(ckv_h, ckv_v, w_sem.at[CKV], p, u * 8 + t, 0)
                fetch(ckv_h, ckv_v, w_sem.at[CKV], p + _NC // 4, u * 8 + t, 1)

        @pl.when(u == 2)
        def _():
            for buf, sem in ((xa_v, XA), (xb_v, XB), (wqa_v, WQA), (wqb_v, WQB),
                             (wuk_v, WUK), (wuv_v, WUV), (woa_v, WOA)):
                wait_all(buf, w_sem.at[sem])

        @pl.when(jnp.logical_and(u >= 2, u < 2 + _H // _G))
        def _():
            a_query(u - 2)

    a_regroup_query()

    lag = _NBUF - 1
    n_split_q = _M // _NW // _CW
    n_split_c = _C // _NW // _CW
    t_split_k = n_split_q
    t_split_v = t_split_k + n_split_c
    t_query = t_split_v + n_split_c
    t_attend = t_query + _H + 1
    t_value = t_attend + _B * per_group + 1
    assert t_value + _H <= n_steps

    def during(i, start, n, fn):
        @pl.when(jnp.logical_and(i >= start, i < start + n))
        def _():
            fn(i - start)

    @pl.loop(0, n_steps + lag)
    def _(i):
        during(i, 0, n_steps, fetch_kv)

        @pl.when(i >= n_steps)
        def _():
            @pl.loop(0, 2)
            def _(u):
                fetch_wob((i - n_steps) * 2 + u)

        during(i, lag, n_steps, a_attend)

        during(i, 0, n_split_q, lambda t: b_split_heads(wqb_v, wqh_s, t))
        during(i, t_split_k, n_split_c, lambda t: b_split_heads(wuk_v, wkh_s, t))
        during(i, t_split_v, n_split_c, lambda t: b_split_heads(wuv_v, wvh_s, t))
        during(i, t_query, _H, b_query)

        @pl.when(i == t_attend - 1)
        def _():
            b_regroup_query()
            wait_all(ckv_v, w_sem.at[CKV])

        during(i, t_attend, _B * per_group, b_attend)

        @pl.when(i == t_value - 1)
        def _():
            b_regroup_ctx()

        during(i, t_value, _H, b_value)

    @pl.loop(2 * lag, _H // _NW)
    def _(u):
        fetch_wob(u)

    a_regroup_out()
    zero = jnp.zeros((_R, _M), _F32)
    out_a = lax.fori_loop(0, _H // _G, lambda u, acc: acc + a_project(u), zero)
    out_b = lax.fori_loop(0, 2 * _H // _NW, lambda n, acc: acc + b_project(n % 2, n // 2), zero)
    out = jnp.concatenate([out_a, out_b], axis=1)
    out_ref[...] = out[:_B].astype(out_ref.dtype)


@jax.jit
def pallas_concat_heads__mha_block_cached__compressed_kv_cla__decode_kernel(
    A_x: jax.Array,
    A_k_cache: jax.Array,
    A_v_cache: jax.Array,
    A_wq: jax.Array,
    A_wo: jax.Array,
    B_x: jax.Array,
    B_c_kv: jax.Array,
    B_w_q: jax.Array,
    B_w_uk: jax.Array,
    B_w_uv: jax.Array,
    B_w_o: jax.Array,
):
    assert A_k_cache.shape == (_B, _H, _S, _D) and B_c_kv.shape == (_B, _S, _C)
    assert A_x.shape == (_B, 1, _M) and B_x.shape == (_B, 1, _M)

    operands = (
        A_x.reshape(_B, _M),
        A_k_cache.reshape(_B * _H, _S, _D),
        A_v_cache.reshape(_B * _H, _S, _D),
        A_wq.reshape(_NW, _M // _NW, _H * _D),
        A_wo.T.reshape(_NW, _M // _NW, _H * _D),
        B_x.reshape(_B, _M),
        B_c_kv.reshape(_NC, _B * _S // _NC, _C),
        B_w_q.reshape(_NW, _M * _H // _NW, _D),
        B_w_uk.reshape(_NW, _C * _H // _NW, _D),
        B_w_uv.reshape(_NW, _C * _H // _NW, _D),
        B_w_o.transpose(0, 2, 1).reshape(_NW, _H * _M // _NW, _D),
    )
    resident = [pltpu.VMEM(operands[i].shape, _BF) for i in (3, 4, 6, 7, 8, 9, 10)]
    out = pl.pallas_call(
        _kernel,
        out_shape=jax.ShapeDtypeStruct((_B, 2 * _M), A_x.dtype),
        in_specs=[pl.BlockSpec(memory_space=pltpu.HBM)] * len(operands),
        scratch_shapes=[
            pltpu.VMEM((_B, _M), _BF),
            pltpu.VMEM((_B, _M), _BF),
            pltpu.VMEM((_NBUF, _G, _TK, _D), _BF),
            pltpu.VMEM((_NBUF, _G, _TK, _D), _BF),
            *resident,
            pltpu.VMEM((_CW * _H // 2, _D), jnp.uint32),
            pltpu.VMEM((_H, _M, _D), _BF),
            pltpu.VMEM((_H, _C, _D), _BF),
            pltpu.VMEM((_H, _C, _D), _BF),
            pltpu.VMEM((_H * _R, _D), _F32),
            pltpu.VMEM((_B * _H, _D), _F32),
            pltpu.VMEM((_G, _D), _F32),
            pltpu.VMEM((_G, _D), _F32),
            pltpu.VMEM((_G, _D), _F32),
            pltpu.VMEM((_B * _H, _D), _F32),
            pltpu.VMEM((_C // _D, _H * _R, _D), _F32),
            pltpu.VMEM((_B * _H, _C), _BF),
            pltpu.VMEM((_H, _D), _F32),
            pltpu.VMEM((_H, _D), _F32),
            pltpu.VMEM((_H, _C), _F32),
            pltpu.VMEM((_C // _D, _B * _H, _D), _F32),
            pltpu.VMEM((_C // _D, _H * _R, _D), _F32),
            pltpu.VMEM((_H, _R, _D), _F32),
            pltpu.SemaphoreType.DMA((2, _NBUF)),
            pltpu.SemaphoreType.DMA((8,)),
            pltpu.SemaphoreType.DMA((2, _H // _NW)),
        ],
        compiler_params=pltpu.CompilerParams(vmem_limit_bytes=100 * 1024 * 1024),
    )(*operands)
    return out.reshape(_B, 1, 2 * _M)
```

```python
import jax
import jax.numpy as jnp
from jax import lax
import jax.experimental.pallas as pl
import jax.experimental.pallas.tpu as pltpu

_BF = jnp.bfloat16
_F32 = jnp.float32
_NT = (((1,), (1,)), ((), ()))
_NN = (((1,), (0,)), ((), ()))

_B = 4
_H = 32
_S = 4096
_D = 128
_M = 576
_C = 512
_R = 8

_G = 8
_TK = 512
_NBUF = 4
_SEG = 64
_NW = 4
_NC = 16
_CW = 16


def _dot(a, b, dims):
    return lax.dot_general(a, b, dims, preferred_element_type=_F32)


def _tile(start, size):
    return pl.ds(pl.multiple_of(start * size, size), size)


def _kernel(xa_h, k_h, v_h, wqa_h, woa_h, xb_h, ckv_h, wqb_h, wuk_h, wuv_h, wob_h,
            out_ref,
            xa_v, xb_v, k_v, v_v, wqa_v, woa_v, ckv_v, wqb_v, wuk_v, wuv_v, wob_v,
            word_s, wqh_s, wkh_s, wvh_s,
            qah_s, qa_s, ma_s, la_s, acca_s, oa_s, outa_s,
            qh_s, qc_s, mb_s, lb_s, accb_s, cc_s, ch_s, ctx_s,
            kv_sem, w_sem, wob_sem):
    scale = _D ** -0.5
    per_group = _S // _TK
    n_steps = _B * _H // _G * per_group
    XA, XB, WQA, WQB, WUK, WUV, CKV, WOA = range(8)

    def copy(src, dst, sem, prio):
        pltpu.make_async_copy(src, dst, sem).start(priority=prio)

    def wait_all(buf, sem):
        pltpu.make_async_copy(buf, buf, sem).wait()

    def fetch(src, dst, sem, pair, t, prio):
        cols = src.shape[2]
        if cols <= _C:
            idx = (pl.ds(2 * pair, 2), _tile(t, _SEG * _D // cols))
        else:
            per_row = cols * 8 // (_SEG * _D)
            idx = (pl.ds(2 * pair, 2), _tile(t // per_row, 8), _tile(t % per_row, cols // per_row))
        copy(src.at[idx], dst.at[idx], sem, prio)

    def fetch_kv(i):
        slot = i % _NBUF
        group = i // per_group
        head0 = group % _B * _H + group // _B * _G
        seg0 = i % per_group * (_TK // _SEG)

        @pl.loop(0, _TK // _SEG)
        def _(t):
            for p in range(_G // 2):
                src = (pl.ds(head0 + 2 * p, 2), _tile(seg0 + t, _SEG))
                dst = (slot, pl.ds(2 * p, 2), _tile(t, _SEG))
                copy(k_h.at[src], k_v.at[dst], kv_sem.at[0, slot], 0)
                copy(v_h.at[src], v_v.at[dst], kv_sem.at[1, slot], 1)

    def fetch_wob(u):
        per_head = _M // _SEG

        @pl.loop(0, per_head)
        def _(t):
            for p in range(2):
                fetch(wob_h, wob_v, wob_sem.at[p, u], p, u * per_head + t, p)

    def pad_rows(x):
        x = x.astype(_F32)
        return jnp.concatenate([x, jnp.zeros_like(x)], axis=0)

    def a_query(u):
        w = wqa_v[:, :, _tile(u, _G * _D)].reshape(_M, _G * _D)
        q = _dot(pad_rows(xa_v[...]).astype(_BF), w, _NN)
        for h in range(_G):
            qah_s[pl.ds(h * _R, _R), :] = q[:, h * _D:(h + 1) * _D]
        for b in range(_B):
            qa_s[u * _B + b] = qah_s[pl.ds(b, _G, stride=_R), :]

    def a_attend(i):
        slot = i % _NBUF
        group = i // per_group

        @pl.when(i % per_group == 0)
        def _():
            ma_s[...] = jnp.full(ma_s.shape, -jnp.inf, _F32)
            la_s[...] = jnp.zeros(la_s.shape, _F32)
            acca_s[...] = jnp.zeros(acca_s.shape, _F32)

        wait_all(k_v.at[slot], kv_sem.at[0, slot])
        wait_all(v_v.at[slot], kv_sem.at[1, slot])

        def own_rows(lhs, rhs_ref, dims):
            res = _dot(lhs, rhs_ref[slot, 0], dims)
            row = lax.broadcasted_iota(jnp.int32, res.shape, 0)
            for h in range(1, _G):
                res = jnp.where(row == h, _dot(lhs, rhs_ref[slot, h], dims), res)
            return res

        s = own_rows(qa_s[group].astype(_BF), k_v, _NT) * scale
        m_old = ma_s[...]
        m_new = jnp.maximum(m_old, jnp.max(s, axis=1, keepdims=True))
        alpha = jnp.exp(m_old - m_new)
        p = jnp.exp(s - m_new[:, :1])
        l_new = alpha * la_s[...] + jnp.sum(p, axis=1, keepdims=True)
        acc = alpha * acca_s[...] + own_rows(p.astype(_BF), v_v, _NN)
        ma_s[...] = m_new
        la_s[...] = l_new
        acca_s[...] = acc
        oa_s[_tile(group % _B, _G), :] = acc / l_new

        @pl.when((i + 1) % (_B * per_group) == 0)
        def _():
            o = jnp.concatenate(
                [pad_rows(oa_s[pl.ds(h, _B, stride=_G), :]) for h in range(_G)], axis=1)
            w = woa_v[:, :, _tile(group // _B, _G * _D)].reshape(_M, _G * _D)
            outa_s[...] += _dot(o.astype(_BF), w, _NT)

    def b_split_heads(w_v, wh_s, t):
        per_range = w_v.shape[1] // (_CW * _H)

        @pl.loop(0, _NW)
        def _(r):
            word_s[...] = pltpu.bitcast(w_v[r, _tile(t, _CW * _H), :], jnp.uint32)
            cs = _tile(r * per_range + t, _CW)
            for j in range(_H // 2):
                u = word_s[pl.ds(j, _CW, stride=_H // 2), :]
                wh_s[2 * j, cs, :] = pltpu.bitcast(u << 16, _F32).astype(_BF)
                wh_s[2 * j + 1, cs, :] = pltpu.bitcast(
                    u & jnp.uint32(0xFFFF0000), _F32).astype(_BF)

    def b_query(h):
        q = _dot(pad_rows(xb_v[...]).astype(_BF), wqh_s[h], _NN)
        q = _dot(q.astype(_BF), wkh_s[h], _NT)
        for c in range(_C // _D):
            qh_s[c, _tile(h, _R), :] = q[:, c * _D:(c + 1) * _D]

    def b_regroup_query():
        for b in range(_B):
            for c in range(_C // _D):
                qc_s[pl.ds(b * _H, _H), pl.ds(c * _D, _D)] = (
                    qh_s[c, pl.ds(b, _H, stride=_R), :].astype(_BF))

    def b_attend(t):
        hs = _tile(t // per_group, _H)
        per_range = ckv_v.shape[1] // _TK

        @pl.when(t % per_group == 0)
        def _():
            mb_s[...] = jnp.full(mb_s.shape, -jnp.inf, _F32)
            lb_s[...] = jnp.zeros(lb_s.shape, _F32)
            accb_s[...] = jnp.zeros(accb_s.shape, _F32)

        lat = ckv_v[t // per_range, _tile(t % per_range, _TK), :]
        s = _dot(qc_s[hs, :], lat, _NT) * scale
        m_old = mb_s[...]
        m_new = jnp.maximum(m_old, jnp.max(s, axis=1, keepdims=True))
        alpha = jnp.exp(m_old - m_new)
        p = jnp.exp(s - m_new[:, :1])
        l_new = alpha * lb_s[...] + jnp.sum(p, axis=1, keepdims=True)
        acc = alpha[:, :1] * accb_s[...] + _dot(p.astype(_BF), lat, _NN)
        mb_s[...] = m_new
        lb_s[...] = l_new
        accb_s[...] = acc
        for c in range(_C // _D):
            cc_s[c, hs, :] = acc[:, c * _D:(c + 1) * _D] / l_new

    def b_regroup_ctx():
        @pl.loop(0, _C // _D)
        def _(c):
            for h in range(_H):
                ch_s[c, pl.ds(h * _R, _R), :] = pad_rows(cc_s[c, pl.ds(h, _B, stride=_H), :])

    def b_value(h):
        lat = jnp.concatenate([ch_s[c, _tile(h, _R), :] for c in range(_C // _D)], axis=1)
        ctx_s[h] = _dot(lat.astype(_BF), wvh_s[h], _NN)

    def b_project(p, u):
        rows = _tile(u, _M)
        wait_all(wob_v.at[pl.ds(2 * p, 2), rows], wob_sem.at[p, u])
        parts = [_dot(ctx_s[r * (_H // _NW) + u].astype(_BF), wob_v[r, rows, :], _NT)
                 for r in (2 * p, 2 * p + 1)]
        return parts[0] + parts[1]

    n_wide = _M * _H // _NW // _SEG
    n_narrow = _C * _H // _NW // _SEG

    @pl.loop(0, n_wide)
    def _(t):
        for p in range(_NW // 2):
            fetch(wqa_h, wqa_v, w_sem.at[WQA], p, t, 0)
            fetch(wqb_h, wqb_v, w_sem.at[WQB], p, t, 1)

        @pl.when(t < n_narrow)
        def _():
            for p in range(_NW // 2):
                fetch(wuk_h, wuk_v, w_sem.at[WUK], p, t, 0)
                fetch(wuv_h, wuv_v, w_sem.at[WUV], p, t, 1)

        for p in range(_NW // 2):
            fetch(woa_h, woa_v, w_sem.at[WOA], p, t, p)

    copy(xa_h, xa_v, w_sem.at[XA], 0)
    copy(xb_h, xb_v, w_sem.at[XB], 1)

    @pl.loop(0, 8)
    def _(u):
        @pl.loop(0, 8)
        def _(t):
            for p in range(_NC // 4):
                fetch(ckv_h, ckv_v, w_sem.at[CKV], p, u * 8 + t, 0)
                fetch(ckv_h, ckv_v, w_sem.at[CKV], p + _NC // 4, u * 8 + t, 1)

        @pl.when(u == 2)
        def _():
            for buf, sem in ((xa_v, XA), (xb_v, XB), (wqa_v, WQA), (wqb_v, WQB),
                             (wuk_v, WUK), (wuv_v, WUV), (woa_v, WOA)):
                wait_all(buf, w_sem.at[sem])

        @pl.when(jnp.logical_and(u >= 2, u < 2 + _H // _G))
        def _():
            a_query(u - 2)

    outa_s[...] = jnp.zeros(outa_s.shape, _F32)

    lag = _NBUF - 1
    n_split_q = _M // _NW // _CW
    n_split_c = _C // _NW // _CW
    t_split_k = n_split_q
    t_split_v = t_split_k + n_split_c
    t_query = t_split_v + n_split_c
    t_attend = t_query + _H + 1
    t_value = t_attend + _B * per_group + 1
    assert t_value + _H <= n_steps

    def during(i, start, n, fn):
        @pl.when(jnp.logical_and(i >= start, i < start + n))
        def _():
            fn(i - start)

    @pl.loop(0, n_steps + lag)
    def _(i):
        during(i, 0, n_steps, fetch_kv)
        during(i, n_steps - 1, lag + 1, fetch_wob)
        during(i, lag, n_steps, a_attend)

        during(i, 0, n_split_q, lambda t: b_split_heads(wqb_v, wqh_s, t))
        during(i, t_split_k, n_split_c, lambda t: b_split_heads(wuk_v, wkh_s, t))
        during(i, t_split_v, n_split_c, lambda t: b_split_heads(wuv_v, wvh_s, t))
        during(i, t_query, _H, b_query)

        @pl.when(i == t_attend - 1)
        def _():
            b_regroup_query()
            wait_all(ckv_v, w_sem.at[CKV])

        during(i, t_attend, _B * per_group, b_attend)

        @pl.when(i == t_value - 1)
        def _():
            b_regroup_ctx()

        during(i, t_value, _H, b_value)

    def project(n, acc):
        during(n, -(lag + 1), _H // _NW, fetch_wob)
        return acc + b_project(n % 2, n // 2)

    out_b = lax.fori_loop(0, 2 * _H // _NW, project, jnp.zeros((_R, _M), _F32))
    out = jnp.concatenate([outa_s[...], out_b], axis=1)
    out_ref[...] = out[:_B].astype(out_ref.dtype)


def _scoped_kernel(*refs):
    pl.run_scoped(
        lambda *sems: _kernel(*refs, *sems),
        pltpu.SemaphoreType.DMA((2, _NBUF)),
        pltpu.SemaphoreType.DMA((8,)),
        pltpu.SemaphoreType.DMA((2, _H // _NW)),
    )


@jax.jit
def pallas_concat_heads__mha_block_cached__compressed_kv_cla__decode_kernel(
    A_x: jax.Array,
    A_k_cache: jax.Array,
    A_v_cache: jax.Array,
    A_wq: jax.Array,
    A_wo: jax.Array,
    B_x: jax.Array,
    B_c_kv: jax.Array,
    B_w_q: jax.Array,
    B_w_uk: jax.Array,
    B_w_uv: jax.Array,
    B_w_o: jax.Array,
):
    assert A_k_cache.shape == (_B, _H, _S, _D) and B_c_kv.shape == (_B, _S, _C)
    assert A_x.shape == (_B, 1, _M) and B_x.shape == (_B, 1, _M)

    operands = (
        A_x.reshape(_B, _M),
        A_k_cache.reshape(_B * _H, _S, _D),
        A_v_cache.reshape(_B * _H, _S, _D),
        A_wq.reshape(_NW, _M // _NW, _H * _D),
        A_wo.T.reshape(_NW, _M // _NW, _H * _D),
        B_x.reshape(_B, _M),
        B_c_kv.reshape(_NC, _B * _S // _NC, _C),
        B_w_q.reshape(_NW, _M * _H // _NW, _D),
        B_w_uk.reshape(_NW, _C * _H // _NW, _D),
        B_w_uv.reshape(_NW, _C * _H // _NW, _D),
        B_w_o.transpose(0, 2, 1).reshape(_NW, _H * _M // _NW, _D),
    )
    resident = [pltpu.VMEM(operands[i].shape, _BF) for i in (3, 4, 6, 7, 8, 9, 10)]
    out = pl.pallas_call(
        _scoped_kernel,
        out_shape=jax.ShapeDtypeStruct((_B, 2 * _M), A_x.dtype),
        in_specs=[pl.BlockSpec(memory_space=pltpu.HBM)] * len(operands),
        scratch_shapes=[
            pltpu.VMEM((_B, _M), _BF),
            pltpu.VMEM((_B, _M), _BF),
            pltpu.VMEM((_NBUF, _G, _TK, _D), _BF),
            pltpu.VMEM((_NBUF, _G, _TK, _D), _BF),
            *resident,
            pltpu.VMEM((_CW * _H // 2, _D), jnp.uint32),
            pltpu.VMEM((_H, _M, _D), _BF),
            pltpu.VMEM((_H, _C, _D), _BF),
            pltpu.VMEM((_H, _C, _D), _BF),
            pltpu.VMEM((_G * _R, _D), _F32),
            pltpu.VMEM((_B * _H // _G, _G, _D), _F32),
            pltpu.VMEM((_G, _D), _F32),
            pltpu.VMEM((_G, _D), _F32),
            pltpu.VMEM((_G, _D), _F32),
            pltpu.VMEM((_B * _G, _D), _F32),
            pltpu.VMEM((_R, _M), _F32),
            pltpu.VMEM((_C // _D, _H * _R, _D), _F32),
            pltpu.VMEM((_B * _H, _C), _BF),
            pltpu.VMEM((_H, _D), _F32),
            pltpu.VMEM((_H, _D), _F32),
            pltpu.VMEM((_H, _C), _F32),
            pltpu.VMEM((_C // _D, _B * _H, _D), _F32),
            pltpu.VMEM((_C // _D, _H * _R, _D), _F32),
            pltpu.VMEM((_H, _R, _D), _F32),
        ],
        compiler_params=pltpu.CompilerParams(vmem_limit_bytes=100 * 1024 * 1024),
    )(*operands)
    return out.reshape(_B, 1, 2 * _M)
```

```python
import jax
import jax.numpy as jnp
from jax import lax
import jax.experimental.pallas as pl
import jax.experimental.pallas.tpu as pltpu

_BF = jnp.bfloat16
_F32 = jnp.float32
_NT = (((1,), (1,)), ((), ()))
_NN = (((1,), (0,)), ((), ()))

_B = 4
_H = 32
_S = 4096
_D = 128
_M = 576
_C = 512
_R = 8

_G = 8
_TK = 512
_NBUF = 4
_SEG = 64
_NW = 4
_NC = 16
_PAD = _M % 128
_CW = 16


def _dot(a, b, dims):
    return lax.dot_general(a, b, dims, preferred_element_type=_F32)


def _tile(start, size):
    return pl.ds(pl.multiple_of(start * size, size), size)


def _kernel(xa_h, k_h, v_h, wqa_h, woa_h, xb_h, ckv_h, wqb_h, wuk_h, wuv_h, wob_h,
            out_ref,
            xa_v, xb_v, k_v, v_v, wqa_v, woa_v, ckv_v, wqb_v, wuk_v, wuv_v, wob_v,
            word_s, wqh_s, wkh_s, wvh_s,
            qah_s, qa_s, ma_s, la_s, acca_s, oa_s, outa_s,
            qh_s, qc_s, mb_s, lb_s, accb_s, cc_s, ch_s, ctx_s,
            kv_sem, w_sem, wob_sem):
    scale = _D ** -0.5
    per_group = _S // _TK
    n_steps = _B * _H // _G * per_group
    XA, XB, WQA, WQB, WUK, WUV, CKV, WOA = range(8)

    def copy(src, dst, sem, prio):
        pltpu.make_async_copy(src, dst, sem).start(priority=prio)

    def wait_all(buf, sem):
        pltpu.make_async_copy(buf, buf, sem).wait()

    def fetch(src, dst, sem, pair, t, prio):
        idx = (pl.ds(2 * pair, 2), _tile(t, _SEG * _D // src.shape[2]))
        copy(src.at[idx], dst.at[idx], sem, prio)

    def fetch_wide(src, dst, sem, pair, row, col, prio):
        idx = (pl.ds(2 * pair, 2), _tile(row, 8), _tile(col, _SEG * _D // 8))
        copy(src.at[idx], dst.at[idx], sem, prio)

    def fetch_kv(i):
        slot = i % _NBUF
        group = i // per_group
        head0 = group % _B * _H + group // _B * _G
        seg0 = i % per_group * (_TK // _SEG)

        @pl.loop(0, _TK // _SEG)
        def _(t):
            for p in range(_G // 2):
                src = (pl.ds(head0 + 2 * p, 2), _tile(seg0 + t, _SEG))
                dst = (slot, pl.ds(2 * p, 2), _tile(t, _SEG))
                copy(k_h.at[src], k_v.at[dst], kv_sem.at[0, slot], 0)
                copy(v_h.at[src], v_v.at[dst], kv_sem.at[1, slot], 1)

    def fetch_wob(u):
        per_head = _M // _SEG

        @pl.loop(0, per_head)
        def _(t):
            for p in range(2):
                fetch(wob_h, wob_v, wob_sem.at[p, u], p, u * per_head + t, p)

    def pad_rows(x):
        x = x.astype(_F32)
        return jnp.concatenate([x, jnp.zeros_like(x)], axis=0)

    def a_query(u):
        w = wqa_v[:, :, _tile(u, _G * _D)].reshape(_M, _G * _D)
        q = _dot(pad_rows(xa_v[...]).astype(_BF), w, _NN)
        for h in range(_G):
            qah_s[pl.ds(h * _R, _R), :] = q[:, h * _D:(h + 1) * _D]
        for b in range(_B):
            qa_s[u * _B + b] = qah_s[pl.ds(b, _G, stride=_R), :]

    def a_attend(i):
        slot = i % _NBUF
        group = i // per_group

        @pl.when(i % per_group == 0)
        def _():
            ma_s[...] = jnp.full(ma_s.shape, -jnp.inf, _F32)
            la_s[...] = jnp.zeros(la_s.shape, _F32)
            acca_s[...] = jnp.zeros(acca_s.shape, _F32)

        def own_rows(lhs, rhs_ref, dims):
            res = _dot(lhs, rhs_ref[slot, 0], dims)
            row = lax.broadcasted_iota(jnp.int32, res.shape, 0)
            for h in range(1, _G):
                res = jnp.where(row == h, _dot(lhs, rhs_ref[slot, h], dims), res)
            return res

        wait_all(k_v.at[slot], kv_sem.at[0, slot])
        s = own_rows(qa_s[group].astype(_BF), k_v, _NT) * scale
        m_old = ma_s[...]
        m_new = jnp.maximum(m_old, jnp.max(s, axis=1, keepdims=True))
        alpha = jnp.exp(m_old - m_new)
        p = jnp.exp(s - m_new[:, :1])
        l_new = alpha * la_s[...] + jnp.sum(p, axis=1, keepdims=True)
        wait_all(v_v.at[slot], kv_sem.at[1, slot])
        acc = alpha * acca_s[...] + own_rows(p.astype(_BF), v_v, _NN)
        ma_s[...] = m_new
        la_s[...] = l_new
        acca_s[...] = acc
        oa_s[_tile(group % _B, _G), :] = acc / l_new

        @pl.when((i + 1) % (_B * per_group) == 0)
        def _():
            o = jnp.concatenate(
                [pad_rows(oa_s[pl.ds(h, _B, stride=_G), :]) for h in range(_G)], axis=1)
            w = woa_v[:, :, _tile(group // _B, _G * _D)].reshape(_M, _G * _D)
            outa_s[...] += _dot(o.astype(_BF), w, _NT)

    def b_split_heads(w_v, wh_s, t):
        per_range = w_v.shape[1] // (_CW * _H)

        @pl.loop(0, _NW)
        def _(r):
            word_s[...] = pltpu.bitcast(w_v[r, _tile(t, _CW * _H), :], jnp.uint32)
            cs = _tile(r * per_range + t, _CW)
            for j in range(_H // 2):
                u = word_s[pl.ds(j, _CW, stride=_H // 2), :]
                wh_s[2 * j, cs, :] = pltpu.bitcast(u << 16, _F32).astype(_BF)
                wh_s[2 * j + 1, cs, :] = pltpu.bitcast(
                    u & jnp.uint32(0xFFFF0000), _F32).astype(_BF)

    def b_query(h):
        q = _dot(pad_rows(xb_v[...]).astype(_BF), wqh_s[h], _NN)
        q = _dot(q.astype(_BF), wkh_s[h], _NT)
        for c in range(_C // _D):
            qh_s[c, _tile(h, _R), :] = q[:, c * _D:(c + 1) * _D]

    def b_regroup_query():
        for b in range(_B):
            for c in range(_C // _D):
                qc_s[pl.ds(b * _H, _H), pl.ds(c * _D, _D)] = (
                    qh_s[c, pl.ds(b, _H, stride=_R), :].astype(_BF))

    def b_attend(t):
        hs = _tile(t // per_group, _H)
        per_range = ckv_v.shape[1] // _TK

        @pl.when(t % per_group == 0)
        def _():
            mb_s[...] = jnp.full(mb_s.shape, -jnp.inf, _F32)
            lb_s[...] = jnp.zeros(lb_s.shape, _F32)
            accb_s[...] = jnp.zeros(accb_s.shape, _F32)

        lat = ckv_v[t // per_range, _tile(t % per_range, _TK), :]
        s = _dot(qc_s[hs, :], lat, _NT) * scale
        m_old = mb_s[...]
        m_new = jnp.maximum(m_old, jnp.max(s, axis=1, keepdims=True))
        alpha = jnp.exp(m_old - m_new)
        p = jnp.exp(s - m_new[:, :1])
        l_new = alpha * lb_s[...] + jnp.sum(p, axis=1, keepdims=True)
        acc = alpha[:, :1] * accb_s[...] + _dot(p.astype(_BF), lat, _NN)
        mb_s[...] = m_new
        lb_s[...] = l_new
        accb_s[...] = acc
        for c in range(_C // _D):
            cc_s[c, hs, :] = acc[:, c * _D:(c + 1) * _D] / l_new

    def b_regroup_ctx():
        @pl.loop(0, _C // _D)
        def _(c):
            for h in range(_H):
                ch_s[c, pl.ds(h * _R, _R), :] = pad_rows(cc_s[c, pl.ds(h, _B, stride=_H), :])

    def b_value(h):
        lat = jnp.concatenate([ch_s[c, _tile(h, _R), :] for c in range(_C // _D)], axis=1)
        ctx_s[h] = _dot(lat.astype(_BF), wvh_s[h], _NN)

    def b_project(acc, chunks):
        for p, u in chunks:
            wait_all(wob_v.at[pl.ds(2 * p, 2), _tile(u, _M)], wob_sem.at[p, u])
        for p, u in chunks:
            for r in (2 * p, 2 * p + 1):
                w = wob_v[r, _tile(u, _M), :]
                w = jnp.concatenate([w[:_PAD], w], axis=0)
                acc = acc + _dot(ctx_s[r * (_H // _NW) + u].astype(_BF), w, _NT)
        return acc

    @pl.loop(0, _M // _NW // 8)
    def _(row):
        @pl.loop(0, 4)
        def _(col):
            for p in range(_NW // 2):
                fetch_wide(wqa_h, wqa_v, w_sem.at[WQA], p, row, col, 0)
                fetch(wqb_h, wqb_v, w_sem.at[WQB], p, row * 4 + col, 1)

            @pl.when(row < _C // _NW // 8)
            def _():
                t = jnp.minimum(row, _C // _NW // 8 - 1) * 4 + col
                for p in range(_NW // 2):
                    fetch(wuk_h, wuk_v, w_sem.at[WUK], p, t, 0)
                    fetch(wuv_h, wuv_v, w_sem.at[WUV], p, t, 1)

            for p in range(_NW // 2):
                fetch_wide(woa_h, woa_v, w_sem.at[WOA], p, row, col, p)

    copy(xa_h, xa_v, w_sem.at[XA], 0)
    copy(xb_h, xb_v, w_sem.at[XB], 1)

    @pl.loop(0, 8)
    def _(u):
        @pl.loop(0, 8)
        def _(t):
            for p in range(_NC // 4):
                fetch(ckv_h, ckv_v, w_sem.at[CKV], p, u * 8 + t, 0)
                fetch(ckv_h, ckv_v, w_sem.at[CKV], p + _NC // 4, u * 8 + t, 1)

        @pl.when(u == 2)
        def _():
            for buf, sem in ((xa_v, XA), (xb_v, XB), (wqa_v, WQA), (wqb_v, WQB),
                             (wuk_v, WUK), (wuv_v, WUV), (woa_v, WOA)):
                wait_all(buf, w_sem.at[sem])

        @pl.when(jnp.logical_and(u >= 2, u < 2 + _H // _G))
        def _():
            a_query(u - 2)

    outa_s[...] = jnp.zeros(outa_s.shape, _F32)

    lag = _NBUF - 1
    n_split_q = _M // _NW // _CW
    n_split_c = _C // _NW // _CW
    t_split_k = n_split_q
    t_split_v = t_split_k + n_split_c
    t_query = t_split_v + n_split_c
    t_attend = t_query + _H + 1
    t_value = t_attend + _B * per_group + 1
    assert t_value + _H <= n_steps

    def during(i, start, n, fn):
        @pl.when(jnp.logical_and(i >= start, i < start + n))
        def _():
            fn(jnp.clip(i - start, 0, n - 1))

    @pl.loop(0, n_steps + lag)
    def _(i):
        during(i, 0, n_steps, fetch_kv)
        during(i, n_steps - 1, lag + 1, fetch_wob)
        during(i, lag, n_steps, a_attend)

        during(i, 0, n_split_q, lambda t: b_split_heads(wqb_v, wqh_s, t))
        during(i, t_split_k, n_split_c, lambda t: b_split_heads(wuk_v, wkh_s, t))
        during(i, t_split_v, n_split_c, lambda t: b_split_heads(wuv_v, wvh_s, t))
        during(i, t_query, _H, b_query)

        @pl.when(i == t_attend - 1)
        def _():
            b_regroup_query()
            wait_all(ckv_v, w_sem.at[CKV])

        during(i, t_attend, _B * per_group, b_attend)

        @pl.when(i == t_value - 1)
        def _():
            b_regroup_ctx()

        during(i, t_value, _H, b_value)

    def project_many(n, acc):
        @pl.loop(0, 2)
        def _(u):
            fetch_wob(lag + 1 + 2 * n + u)

        return b_project(acc, [(0, 3 * n + u) for u in range(3)] + [(1, 2 * n + u) for u in range(2)])

    def project_one(n, acc):
        p = jnp.where(n < 3, n % 2, 1)
        u = jnp.where(n < 3, 6 + n // 2 - 2 * p, n + 2)
        return b_project(acc, [(p, u)])

    assert lag + 1 == 4 and _H // _NW == 8
    out_b = lax.fori_loop(0, 2, project_many, jnp.zeros((_R, _PAD + _M), _F32))
    out_b = lax.fori_loop(0, 6, project_one, out_b)
    out = jnp.concatenate([outa_s[...], out_b[:, _PAD:]], axis=1)
    out_ref[...] = out[:_B].astype(out_ref.dtype)


def _scoped_kernel(*refs):
    pl.run_scoped(
        lambda *sems: _kernel(*refs, *sems),
        pltpu.SemaphoreType.DMA((2, _NBUF)),
        pltpu.SemaphoreType.DMA((8,)),
        pltpu.SemaphoreType.DMA((2, _H // _NW)),
    )


@jax.jit
def pallas_concat_heads__mha_block_cached__compressed_kv_cla__decode_kernel(
    A_x: jax.Array,
    A_k_cache: jax.Array,
    A_v_cache: jax.Array,
    A_wq: jax.Array,
    A_wo: jax.Array,
    B_x: jax.Array,
    B_c_kv: jax.Array,
    B_w_q: jax.Array,
    B_w_uk: jax.Array,
    B_w_uv: jax.Array,
    B_w_o: jax.Array,
):
    assert A_k_cache.shape == (_B, _H, _S, _D) and B_c_kv.shape == (_B, _S, _C)
    assert A_x.shape == (_B, 1, _M) and B_x.shape == (_B, 1, _M)

    operands = (
        A_x.reshape(_B, _M),
        A_k_cache.reshape(_B * _H, _S, _D),
        A_v_cache.reshape(_B * _H, _S, _D),
        A_wq.reshape(_NW, _M // _NW, _H * _D),
        A_wo.T.reshape(_NW, _M // _NW, _H * _D),
        B_x.reshape(_B, _M),
        B_c_kv.reshape(_NC, _B * _S // _NC, _C),
        B_w_q.reshape(_NW, _M * _H // _NW, _D),
        B_w_uk.reshape(_NW, _C * _H // _NW, _D),
        B_w_uv.reshape(_NW, _C * _H // _NW, _D),
        B_w_o.transpose(0, 2, 1).reshape(_NW, _H * _M // _NW, _D),
    )
    resident = [pltpu.VMEM(operands[i].shape, _BF) for i in (3, 4, 6, 7, 8, 9, 10)]
    out = pl.pallas_call(
        _scoped_kernel,
        out_shape=jax.ShapeDtypeStruct((_B, 2 * _M), A_x.dtype),
        in_specs=[pl.BlockSpec(memory_space=pltpu.HBM)] * len(operands),
        scratch_shapes=[
            pltpu.VMEM((_B, _M), _BF),
            pltpu.VMEM((_B, _M), _BF),
            pltpu.VMEM((_NBUF, _G, _TK, _D), _BF),
            pltpu.VMEM((_NBUF, _G, _TK, _D), _BF),
            *resident,
            pltpu.VMEM((_CW * _H // 2, _D), jnp.uint32),
            pltpu.VMEM((_H, _M, _D), _BF),
            pltpu.VMEM((_H, _C, _D), _BF),
            pltpu.VMEM((_H, _C, _D), _BF),
            pltpu.VMEM((_G * _R, _D), _F32),
            pltpu.VMEM((_B * _H // _G, _G, _D), _F32),
            pltpu.VMEM((_G, _D), _F32),
            pltpu.VMEM((_G, _D), _F32),
            pltpu.VMEM((_G, _D), _F32),
            pltpu.VMEM((_B * _G, _D), _F32),
            pltpu.VMEM((_R, _M), _F32),
            pltpu.VMEM((_C // _D, _H * _R, _D), _F32),
            pltpu.VMEM((_B * _H, _C), _BF),
            pltpu.VMEM((_H, _D), _F32),
            pltpu.VMEM((_H, _D), _F32),
            pltpu.VMEM((_H, _C), _F32),
            pltpu.VMEM((_C // _D, _B * _H, _D), _F32),
            pltpu.VMEM((_C // _D, _H * _R, _D), _F32),
            pltpu.VMEM((_H, _R, _D), _F32),
        ],
        compiler_params=pltpu.CompilerParams(vmem_limit_bytes=100 * 1024 * 1024),
    )(*operands)
    return out.reshape(_B, 1, 2 * _M)
```

```python
import jax
import jax.numpy as jnp
import numpy as np
from jax import lax
import jax.experimental.pallas as pl
import jax.experimental.pallas.tpu as pltpu

_BF = jnp.bfloat16
_F32 = jnp.float32
_LOWEST = float(np.finfo(np.float32).min)
_NT = (((1,), (1,)), ((), ()))
_NN = (((1,), (0,)), ((), ()))

_B = 4
_H = 32
_S = 4096
_D = 128
_M = 576
_C = 512
_R = 8

_G = 8
_TK = 512
_NBUF = 4
_SEG = 64
_NW = 4
_NC = 16
_CW = 16
_PAD = _M % 128


def _dot(a, b, dims):
    return lax.dot_general(a, b, dims, preferred_element_type=_F32)


def _tile(start, size):
    return pl.ds(pl.multiple_of(start * size, size), size)


def _kernel(xa_h, k_h, v_h, wqa_h, woa_h, xb_h, ckv_h, wqb_h, wuk_h, wuv_h, wob_h,
            out_ref,
            xa_v, xb_v, k_v, v_v, wqa_v, woa_v, ckv_v, wqb_v, wuk_v, wuv_v, wob_v,
            word_s, wqh_s, wkh_s, wvh_s,
            qah_s, qa_s, ma_s, la_s, acca_s, oa_s, outa_s,
            qh_s, qc_s, mb_s, lb_s, accb_s, cc_s, ch_s, ctx_s,
            kv_sem, w_sem, wob_sem):
    scale = _D ** -0.5
    per_group = _S // _TK
    n_steps = _B * _H // _G * per_group
    XA, XB, WQA, WQB, WUK, WUV, CKV, WOA = range(8)

    def copy(src, dst, sem, prio):
        pltpu.make_async_copy(src, dst, sem).start(priority=prio)

    def wait_all(buf, sem):
        pltpu.make_async_copy(buf, buf, sem).wait()

    def fetch(src, dst, sem, pair, t, prio):
        idx = (pl.ds(2 * pair, 2), _tile(t, _SEG * _D // src.shape[2]))
        copy(src.at[idx], dst.at[idx], sem, prio)

    def fetch_wide(src, dst, sem, pair, row, col, prio):
        idx = (pl.ds(2 * pair, 2), _tile(row, 8), _tile(col, _SEG * _D // 8))
        copy(src.at[idx], dst.at[idx], sem, prio)

    def fetch_kv(i):
        slot = i % _NBUF
        group = i // per_group
        head0 = group % _B * _H + group // _B * _G
        seg0 = i % per_group * (_TK // _SEG)

        @pl.loop(0, _TK // _SEG)
        def _(t):
            for p in range(_G // 2):
                src = (pl.ds(head0 + 2 * p, 2), _tile(seg0 + t, _SEG))
                dst = (slot, pl.ds(2 * p, 2), _tile(t, _SEG))
                copy(k_h.at[src], k_v.at[dst], kv_sem.at[0, slot], 0)
                copy(v_h.at[src], v_v.at[dst], kv_sem.at[1, slot], 1)

    def fetch_wob(u):
        per_head = _M // _SEG

        @pl.loop(0, per_head)
        def _(t):
            for p in range(2):
                fetch(wob_h, wob_v, wob_sem.at[p, u], p, u * per_head + t, p)

    def pad_rows(x):
        x = x.astype(_F32)
        return jnp.concatenate([x, jnp.zeros_like(x)], axis=0)

    def a_query(u):
        w = wqa_v[:, :, _tile(u, _G * _D)].reshape(_M, _G * _D)
        q = _dot(pad_rows(xa_v[...]).astype(_BF), w, _NN)
        for h in range(_G):
            qah_s[pl.ds(h * _R, _R), :] = q[:, h * _D:(h + 1) * _D]
        for b in range(_B):
            qa_s[u * _B + b] = qah_s[pl.ds(b, _G, stride=_R), :]

    def a_attend(i):
        slot = i % _NBUF
        group = i // per_group

        @pl.when(i % per_group == 0)
        def _():
            ma_s[...] = jnp.full(ma_s.shape, _LOWEST, _F32)
            la_s[...] = jnp.zeros(la_s.shape, _F32)
            acca_s[...] = jnp.zeros(acca_s.shape, _F32)

        def own_rows(lhs, rhs_ref, dims):
            res = _dot(lhs, rhs_ref[slot, 0], dims)
            row = lax.broadcasted_iota(jnp.int32, res.shape, 0)
            for h in range(1, _G):
                res = jnp.where(row == h, _dot(lhs, rhs_ref[slot, h], dims), res)
            return res

        wait_all(k_v.at[slot], kv_sem.at[0, slot])
        s = own_rows(qa_s[group].astype(_BF), k_v, _NT) * scale
        m_old = ma_s[...]
        m_new = jnp.maximum(m_old, jnp.max(s, axis=1, keepdims=True))
        alpha = jnp.exp(m_old - m_new)
        p = jnp.exp(s - m_new[:, :1])
        l_new = alpha * la_s[...] + jnp.sum(p, axis=1, keepdims=True)
        wait_all(v_v.at[slot], kv_sem.at[1, slot])
        acc = alpha * acca_s[...] + own_rows(p.astype(_BF), v_v, _NN)
        ma_s[...] = m_new
        la_s[...] = l_new
        acca_s[...] = acc
        oa_s[_tile(group % _B, _G), :] = acc / l_new

        @pl.when((i + 1) % (_B * per_group) == 0)
        def _():
            o = jnp.concatenate(
                [pad_rows(oa_s[pl.ds(h, _B, stride=_G), :]) for h in range(_G)], axis=1)
            w = woa_v[:, :, _tile(group // _B, _G * _D)].reshape(_M, _G * _D)
            outa_s[...] += _dot(o.astype(_BF), w, _NT)

    def b_split_heads(w_v, wh_s, t):
        per_range = w_v.shape[1] // (_CW * _H)

        @pl.loop(0, _NW)
        def _(r):
            word_s[...] = pltpu.bitcast(w_v[r, _tile(t, _CW * _H), :], jnp.uint32)
            cs = _tile(r * per_range + t, _CW)
            for j in range(_H // 2):
                u = word_s[pl.ds(j, _CW, stride=_H // 2), :]
                wh_s[2 * j, cs, :] = pltpu.bitcast(u << 16, _F32).astype(_BF)
                wh_s[2 * j + 1, cs, :] = pltpu.bitcast(
                    u & np.uint32(0xFFFF0000), _F32).astype(_BF)

    def b_query(h):
        q = _dot(pad_rows(xb_v[...]).astype(_BF), wqh_s[h], _NN)
        q = _dot(q.astype(_BF), wkh_s[h], _NT)
        for c in range(_C // _D):
            qh_s[c, _tile(h, _R), :] = q[:, c * _D:(c + 1) * _D]

    def b_regroup_query():
        for b in range(_B):
            for c in range(_C // _D):
                qc_s[pl.ds(b * _H, _H), pl.ds(c * _D, _D)] = (
                    qh_s[c, pl.ds(b, _H, stride=_R), :].astype(_BF))

    def b_attend(t):
        hs = _tile(t // per_group, _H)
        per_range = ckv_v.shape[1] // _TK

        @pl.when(t % per_group == 0)
        def _():
            mb_s[...] = jnp.full(mb_s.shape, _LOWEST, _F32)
            lb_s[...] = jnp.zeros(lb_s.shape, _F32)
            accb_s[...] = jnp.zeros(accb_s.shape, _F32)

        lat = ckv_v[t // per_range, _tile(t % per_range, _TK), :]
        s = _dot(qc_s[hs, :], lat, _NT) * scale
        m_old = mb_s[...]
        m_new = jnp.maximum(m_old, jnp.max(s, axis=1, keepdims=True))
        alpha = jnp.exp(m_old - m_new)
        p = jnp.exp(s - m_new[:, :1])
        l_new = alpha * lb_s[...] + jnp.sum(p, axis=1, keepdims=True)
        acc = alpha[:, :1] * accb_s[...] + _dot(p.astype(_BF), lat, _NN)
        mb_s[...] = m_new
        lb_s[...] = l_new
        accb_s[...] = acc
        for c in range(_C // _D):
            cc_s[c, hs, :] = acc[:, c * _D:(c + 1) * _D] / l_new

    def b_regroup_ctx():
        @pl.loop(0, _C // _D)
        def _(c):
            for h in range(_H):
                ch_s[c, pl.ds(h * _R, _R), :] = pad_rows(cc_s[c, pl.ds(h, _B, stride=_H), :])

    def b_value(h):
        lat = jnp.concatenate([ch_s[c, _tile(h, _R), :] for c in range(_C // _D)], axis=1)
        ctx_s[h] = _dot(lat.astype(_BF), wvh_s[h], _NN)

    def b_project(acc, chunks):
        for p, u in chunks:
            wait_all(wob_v.at[pl.ds(2 * p, 2), _tile(u, _M)], wob_sem.at[p, u])
        for p, u in chunks:
            for r in (2 * p, 2 * p + 1):
                w = wob_v[r, _tile(u, _M), :]
                w = jnp.concatenate([w[:_PAD], w], axis=0)
                acc = acc + _dot(ctx_s[r * (_H // _NW) + u].astype(_BF), w, _NT)
        return acc

    @pl.loop(0, _M // _NW // 8)
    def _(row):
        @pl.loop(0, 4)
        def _(col):
            for p in range(_NW // 2):
                fetch_wide(wqa_h, wqa_v, w_sem.at[WQA], p, row, col, 0)
                fetch(wqb_h, wqb_v, w_sem.at[WQB], p, row * 4 + col, 1)

            @pl.when(row < _C // _NW // 8)
            def _():
                t = jnp.minimum(row, _C // _NW // 8 - 1) * 4 + col
                for p in range(_NW // 2):
                    fetch(wuk_h, wuk_v, w_sem.at[WUK], p, t, 0)
                    fetch(wuv_h, wuv_v, w_sem.at[WUV], p, t, 1)

            for p in range(_NW // 2):
                fetch_wide(woa_h, woa_v, w_sem.at[WOA], p, row, col, p)

    copy(xa_h, xa_v, w_sem.at[XA], 0)
    copy(xb_h, xb_v, w_sem.at[XB], 1)

    @pl.loop(0, 8)
    def _(u):
        @pl.loop(0, 8)
        def _(t):
            for p in range(_NC // 4):
                fetch(ckv_h, ckv_v, w_sem.at[CKV], p, u * 8 + t, 0)
                fetch(ckv_h, ckv_v, w_sem.at[CKV], p + _NC // 4, u * 8 + t, 1)

        @pl.when(u == 2)
        def _():
            for buf, sem in ((xa_v, XA), (xb_v, XB), (wqa_v, WQA), (wqb_v, WQB),
                             (wuk_v, WUK), (wuv_v, WUV), (woa_v, WOA)):
                wait_all(buf, w_sem.at[sem])

        @pl.when(jnp.logical_and(u >= 2, u < 2 + _H // _G))
        def _():
            a_query(u - 2)

    outa_s[...] = jnp.zeros(outa_s.shape, _F32)

    lag = _NBUF - 1
    n_split_q = _M // _NW // _CW
    n_split_c = _C // _NW // _CW
    t_split_k = n_split_q
    t_split_v = t_split_k + n_split_c
    t_query = t_split_v + n_split_c
    t_attend = t_query + _H + 1
    t_value = t_attend + _B * per_group + 1
    assert t_value + _H <= n_steps

    def during(i, start, n, fn):
        @pl.when(jnp.logical_and(i >= start, i < start + n))
        def _():
            fn(jnp.clip(i - start, 0, n - 1))

    @pl.loop(0, n_steps + lag)
    def _(i):
        during(i, 0, n_steps, fetch_kv)
        during(i, n_steps - 1, lag + 1, fetch_wob)
        during(i, lag, n_steps, a_attend)

        during(i, 0, n_split_q, lambda t: b_split_heads(wqb_v, wqh_s, t))
        during(i, t_split_k, n_split_c, lambda t: b_split_heads(wuk_v, wkh_s, t))
        during(i, t_split_v, n_split_c, lambda t: b_split_heads(wuv_v, wvh_s, t))
        during(i, t_query, _H, b_query)

        @pl.when(i == t_attend - 1)
        def _():
            b_regroup_query()
            wait_all(ckv_v, w_sem.at[CKV])

        during(i, t_attend, _B * per_group, b_attend)

        @pl.when(i == t_value - 1)
        def _():
            b_regroup_ctx()

        during(i, t_value, _H, b_value)

    def project_many(n, acc):
        return b_project(acc, [(0, 3 * n + u) for u in range(3)]
                         + [(1, 2 * n + u) for u in range(2)])

    def project_one(n, acc):
        p = jnp.where(n < 3, n % 2, 1)
        u = jnp.where(n < 3, 6 + n // 2 - 2 * p, n + 2)
        return b_project(acc, [(p, u)])

    assert _H // _NW == 8
    pl.loop(lag + 1, _H // _NW)(fetch_wob)
    out_b = lax.fori_loop(0, 2, project_many, jnp.zeros((_R, _PAD + _M), _F32))
    out_b = lax.fori_loop(0, 6, project_one, out_b)
    out = jnp.concatenate([outa_s[...], out_b[:, _PAD:]], axis=1)
    out_ref[...] = out[:_B].astype(out_ref.dtype)


def _scoped_kernel(*refs):
    pl.run_scoped(
        lambda *sems: _kernel(*refs, *sems),
        pltpu.SemaphoreType.DMA((2, _NBUF)),
        pltpu.SemaphoreType.DMA((8,)),
        pltpu.SemaphoreType.DMA((2, _H // _NW)),
    )


@jax.jit
def pallas_concat_heads__mha_block_cached__compressed_kv_cla__decode_kernel(
    A_x: jax.Array,
    A_k_cache: jax.Array,
    A_v_cache: jax.Array,
    A_wq: jax.Array,
    A_wo: jax.Array,
    B_x: jax.Array,
    B_c_kv: jax.Array,
    B_w_q: jax.Array,
    B_w_uk: jax.Array,
    B_w_uv: jax.Array,
    B_w_o: jax.Array,
):
    assert A_k_cache.shape == (_B, _H, _S, _D) and B_c_kv.shape == (_B, _S, _C)
    assert A_x.shape == (_B, 1, _M) and B_x.shape == (_B, 1, _M)

    operands = (
        A_x.reshape(_B, _M),
        A_k_cache.reshape(_B * _H, _S, _D),
        A_v_cache.reshape(_B * _H, _S, _D),
        A_wq.reshape(_NW, _M // _NW, _H * _D),
        A_wo.T.reshape(_NW, _M // _NW, _H * _D),
        B_x.reshape(_B, _M),
        B_c_kv.reshape(_NC, _B * _S // _NC, _C),
        B_w_q.reshape(_NW, _M * _H // _NW, _D),
        B_w_uk.reshape(_NW, _C * _H // _NW, _D),
        B_w_uv.reshape(_NW, _C * _H // _NW, _D),
        B_w_o.transpose(0, 2, 1).reshape(_NW, _H * _M // _NW, _D),
    )
    resident = [pltpu.VMEM(operands[i].shape, _BF) for i in (3, 4, 6, 7, 8, 9, 10)]
    out = pl.pallas_call(
        _scoped_kernel,
        out_shape=jax.ShapeDtypeStruct((_B, 2 * _M), A_x.dtype),
        in_specs=[pl.BlockSpec(memory_space=pltpu.HBM)] * len(operands),
        scratch_shapes=[
            pltpu.VMEM((_B, _M), _BF),
            pltpu.VMEM((_B, _M), _BF),
            pltpu.VMEM((_NBUF, _G, _TK, _D), _BF),
            pltpu.VMEM((_NBUF, _G, _TK, _D), _BF),
            *resident,
            pltpu.VMEM((_CW * _H // 2, _D), jnp.uint32),
            pltpu.VMEM((_H, _M, _D), _BF),
            pltpu.VMEM((_H, _C, _D), _BF),
            pltpu.VMEM((_H, _C, _D), _BF),
            pltpu.VMEM((_G * _R, _D), _F32),
            pltpu.VMEM((_B * _H // _G, _G, _D), _F32),
            pltpu.VMEM((_G, _D), _F32),
            pltpu.VMEM((_G, _D), _F32),
            pltpu.VMEM((_G, _D), _F32),
            pltpu.VMEM((_B * _G, _D), _F32),
            pltpu.VMEM((_R, _M), _F32),
            pltpu.VMEM((_C // _D, _H * _R, _D), _F32),
            pltpu.VMEM((_B * _H, _C), _BF),
            pltpu.VMEM((_H, _D), _F32),
            pltpu.VMEM((_H, _D), _F32),
            pltpu.VMEM((_H, _C), _F32),
            pltpu.VMEM((_C // _D, _B * _H, _D), _F32),
            pltpu.VMEM((_C // _D, _H * _R, _D), _F32),
            pltpu.VMEM((_H, _R, _D), _F32),
        ],
        compiler_params=pltpu.CompilerParams(vmem_limit_bytes=100 * 1024 * 1024),
    )(*operands)
    return out.reshape(_B, 1, 2 * _M)
```

```python
import jax
import jax.numpy as jnp
import numpy as np
from jax import lax
import jax.experimental.pallas as pl
import jax.experimental.pallas.tpu as pltpu

_BF = jnp.bfloat16
_F32 = jnp.float32
_LOWEST = float(np.finfo(np.float32).min)
_NT = (((1,), (1,)), ((), ()))
_NN = (((1,), (0,)), ((), ()))

_B = 4
_H = 32
_S = 4096
_D = 128
_M = 576
_C = 512
_R = 8

_G = 8
_TK = 512
_NBUF = 4
_SEG = 64
_NW = 4
_NC = 16
_CW = 16
_PAD = _M % 128


def _dot(a, b, dims):
    return lax.dot_general(a, b, dims, preferred_element_type=_F32)


def _tile(start, size):
    return pl.ds(pl.multiple_of(start * size, size), size)


def _kernel(xa_h, k_h, v_h, wqa_h, woa_h, xb_h, ckv_h, wqb_h, wuk_h, wuv_h, wob_h,
            out_ref,
            xa_v, xb_v, k_v, v_v, wqa_v, woa_v, ckv_v, wqb_v, wuk_v, wuv_v, wob_v,
            word_s, wqh_s, wkh_s, wvh_s,
            qah_s, qa_s, ma_s, la_s, acca_s, oa_s, outa_s,
            qh_s, qc_s, mb_s, lb_s, accb_s, cc_s, ch_s, ctx_s,
            kv_sem, w_sem, wob_sem):
    scale = _D ** -0.5
    per_group = _S // _TK
    n_steps = _B * _H // _G * per_group
    XA, XB, WQA, WQB, WUK, WUV, CKV, WOA = range(8)

    def copy(src, dst, sem, prio):
        pltpu.make_async_copy(src, dst, sem).start(priority=prio)

    def wait_all(buf, sem):
        pltpu.make_async_copy(buf, buf, sem).wait()

    def fetch(src, dst, sem, pair, t, prio):
        idx = (pl.ds(2 * pair, 2), _tile(t, _SEG * _D // src.shape[2]))
        copy(src.at[idx], dst.at[idx], sem, prio)

    def fetch_wide(src, dst, sem, pair, row, col, prio):
        idx = (pl.ds(2 * pair, 2), _tile(row, 8), _tile(col, _SEG * _D // 8))
        copy(src.at[idx], dst.at[idx], sem, prio)

    def fetch_kv(i):
        slot = i % _NBUF
        group = i // per_group
        head0 = group % _B * _H + group // _B * _G
        seg0 = i % per_group * (_TK // _SEG)

        @pl.loop(0, _TK // _SEG)
        def _(t):
            for p in range(_G // 2):
                src = (pl.ds(head0 + 2 * p, 2), _tile(seg0 + t, _SEG))
                dst = (slot, pl.ds(2 * p, 2), _tile(t, _SEG))
                copy(k_h.at[src], k_v.at[dst], kv_sem.at[0, slot], 0)
                copy(v_h.at[src], v_v.at[dst], kv_sem.at[1, slot], 1)

    def fetch_wob(u):
        per_head = _M // _SEG

        @pl.loop(0, per_head)
        def _(t):
            for p in range(2):
                fetch(wob_h, wob_v, wob_sem.at[p, u], p, u * per_head + t, p)

    def pad_rows(x):
        x = x.astype(_F32)
        return jnp.concatenate([x, jnp.zeros_like(x)], axis=0)

    def a_query(u):
        w = wqa_v[:, :, _tile(u, _G * _D)].reshape(_M, _G * _D)
        q = _dot(pad_rows(xa_v[...]).astype(_BF), w, _NN)
        for h in range(_G):
            qah_s[pl.ds(h * _R, _R), :] = q[:, h * _D:(h + 1) * _D]
        for b in range(_B):
            qa_s[u * _B + b] = qah_s[pl.ds(b, _G, stride=_R), :]

    def a_attend(i):
        slot = i % _NBUF
        group = i // per_group

        @pl.when(i % per_group == 0)
        def _():
            ma_s[...] = jnp.full(ma_s.shape, _LOWEST, _F32)
            la_s[...] = jnp.zeros(la_s.shape, _F32)
            acca_s[...] = jnp.zeros(acca_s.shape, _F32)

        def own_rows(lhs, rhs_ref, dims):
            res = _dot(lhs, rhs_ref[slot, 0], dims)
            row = lax.broadcasted_iota(jnp.int32, res.shape, 0)
            for h in range(1, _G):
                res = jnp.where(row == h, _dot(lhs, rhs_ref[slot, h], dims), res)
            return res

        wait_all(k_v.at[slot], kv_sem.at[0, slot])
        s = own_rows(qa_s[group].astype(_BF), k_v, _NT) * scale
        m_old = ma_s[...]
        m_new = jnp.maximum(m_old, jnp.max(s, axis=1, keepdims=True))
        alpha = jnp.exp(m_old - m_new)
        p = jnp.exp(s - m_new[:, :1])
        l_new = alpha * la_s[...] + jnp.sum(p, axis=1, keepdims=True)
        wait_all(v_v.at[slot], kv_sem.at[1, slot])
        acc = alpha * acca_s[...] + own_rows(p.astype(_BF), v_v, _NN)
        ma_s[...] = m_new
        la_s[...] = l_new
        acca_s[...] = acc
        oa_s[_tile(group % _B, _G), :] = acc / l_new

        @pl.when((i + 1) % (_B * per_group) == 0)
        def _():
            o = jnp.concatenate(
                [pad_rows(oa_s[pl.ds(h, _B, stride=_G), :]) for h in range(_G)], axis=1)
            w = woa_v[:, :, _tile(group // _B, _G * _D)].reshape(_M, _G * _D)
            outa_s[...] += _dot(o.astype(_BF), w, _NT)

    def b_split_heads(w_v, wh_s, t):
        per_range = w_v.shape[1] // (_CW * _H)

        @pl.loop(0, _NW)
        def _(r):
            word_s[...] = pltpu.bitcast(w_v[r, _tile(t, _CW * _H), :], jnp.uint32)
            cs = _tile(r * per_range + t, _CW)
            for j in range(_H // 2):
                u = word_s[pl.ds(j, _CW, stride=_H // 2), :]
                wh_s[2 * j, cs, :] = pltpu.bitcast(u << 16, _F32).astype(_BF)
                wh_s[2 * j + 1, cs, :] = pltpu.bitcast(
                    u & np.uint32(0xFFFF0000), _F32).astype(_BF)

    def b_query(h):
        q = _dot(pad_rows(xb_v[...]).astype(_BF), wqh_s[h], _NN)
        q = _dot(q.astype(_BF), wkh_s[h], _NT)
        for c in range(_C // _D):
            qh_s[c, _tile(h, _R), :] = q[:, c * _D:(c + 1) * _D]

    def b_regroup_query():
        for b in range(_B):
            for c in range(_C // _D):
                q = qh_s[c, pl.ds(b, _H, stride=_R), :]
                hi = q.astype(_BF)
                qc_s[b, pl.ds(0, _H), pl.ds(c * _D, _D)] = hi
                qc_s[b, pl.ds(_H, _H), pl.ds(c * _D, _D)] = (q - hi.astype(_F32)).astype(_BF)

    def b_attend(t):
        hs = _tile(t // per_group, _H)
        per_range = ckv_v.shape[1] // _TK

        @pl.when(t % per_group == 0)
        def _():
            mb_s[...] = jnp.full(mb_s.shape, _LOWEST, _F32)
            lb_s[...] = jnp.zeros(lb_s.shape, _F32)
            accb_s[...] = jnp.zeros(accb_s.shape, _F32)

        lat = ckv_v[t // per_range, _tile(t % per_range, _TK), :]
        s = _dot(qc_s[t // per_group], lat, _NT)
        s = (s[:_H] + s[_H:]) * scale
        m_old = mb_s[...]
        m_new = jnp.maximum(m_old, jnp.max(s, axis=1, keepdims=True))
        alpha = jnp.exp(m_old - m_new)
        p = jnp.exp(s - m_new[:, :1])
        l_new = alpha * lb_s[...] + jnp.sum(p, axis=1, keepdims=True)
        acc = alpha[:, :1] * accb_s[...] + _dot(p.astype(_BF), lat, _NN)
        mb_s[...] = m_new
        lb_s[...] = l_new
        accb_s[...] = acc
        for c in range(_C // _D):
            cc_s[c, hs, :] = acc[:, c * _D:(c + 1) * _D] / l_new

    def b_regroup_ctx():
        @pl.loop(0, _C // _D)
        def _(c):
            for h in range(_H):
                ch_s[c, pl.ds(h * _R, _R), :] = pad_rows(cc_s[c, pl.ds(h, _B, stride=_H), :])

    def b_value(h):
        lat = jnp.concatenate([ch_s[c, _tile(h, _R), :] for c in range(_C // _D)], axis=1)
        ctx_s[h] = _dot(lat.astype(_BF), wvh_s[h], _NN)

    def b_project(acc, chunks):
        for p, u in chunks:
            wait_all(wob_v.at[pl.ds(2 * p, 2), _tile(u, _M)], wob_sem.at[p, u])
        for p, u in chunks:
            for r in (2 * p, 2 * p + 1):
                w = wob_v[r, _tile(u, _M), :]
                w = jnp.concatenate([w[:_PAD], w], axis=0)
                acc = acc + _dot(ctx_s[r * (_H // _NW) + u].astype(_BF), w, _NT)
        return acc

    @pl.loop(0, _M // _NW // 8)
    def _(row):
        @pl.loop(0, 4)
        def _(col):
            for p in range(_NW // 2):
                fetch_wide(wqa_h, wqa_v, w_sem.at[WQA], p, row, col, 0)
                fetch(wqb_h, wqb_v, w_sem.at[WQB], p, row * 4 + col, 1)

            @pl.when(row < _C // _NW // 8)
            def _():
                t = jnp.minimum(row, _C // _NW // 8 - 1) * 4 + col
                for p in range(_NW // 2):
                    fetch(wuk_h, wuk_v, w_sem.at[WUK], p, t, 0)
                    fetch(wuv_h, wuv_v, w_sem.at[WUV], p, t, 1)

            for p in range(_NW // 2):
                fetch_wide(woa_h, woa_v, w_sem.at[WOA], p, row, col, p)

    copy(xa_h, xa_v, w_sem.at[XA], 0)
    copy(xb_h, xb_v, w_sem.at[XB], 1)

    @pl.loop(0, 8)
    def _(u):
        @pl.loop(0, 8)
        def _(t):
            for p in range(_NC // 4):
                fetch(ckv_h, ckv_v, w_sem.at[CKV], p, u * 8 + t, 0)
                fetch(ckv_h, ckv_v, w_sem.at[CKV], p + _NC // 4, u * 8 + t, 1)

        @pl.when(u == 2)
        def _():
            for buf, sem in ((xa_v, XA), (xb_v, XB), (wqa_v, WQA), (wqb_v, WQB),
                             (wuk_v, WUK), (wuv_v, WUV), (woa_v, WOA)):
                wait_all(buf, w_sem.at[sem])

        @pl.when(jnp.logical_and(u >= 2, u < 2 + _H // _G))
        def _():
            a_query(u - 2)

    outa_s[...] = jnp.zeros(outa_s.shape, _F32)

    lag = _NBUF - 1
    n_split_q = _M // _NW // _CW
    n_split_c = _C // _NW // _CW
    t_split_k = n_split_q
    t_split_v = t_split_k + n_split_c
    t_query = t_split_v + n_split_c
    t_attend = t_query + _H + 1
    t_value = t_attend + _B * per_group + 1
    assert t_value + _H <= n_steps

    def during(i, start, n, fn):
        @pl.when(jnp.logical_and(i >= start, i < start + n))
        def _():
            fn(jnp.clip(i - start, 0, n - 1))

    @pl.loop(0, n_steps + lag)
    def _(i):
        during(i, 0, n_steps, fetch_kv)
        during(i, n_steps - 1, lag + 1, fetch_wob)
        during(i, lag, n_steps, a_attend)

        during(i, 0, n_split_q, lambda t: b_split_heads(wqb_v, wqh_s, t))
        during(i, t_split_k, n_split_c, lambda t: b_split_heads(wuk_v, wkh_s, t))
        during(i, t_split_v, n_split_c, lambda t: b_split_heads(wuv_v, wvh_s, t))
        during(i, t_query, _H, b_query)

        @pl.when(i == t_attend - 1)
        def _():
            b_regroup_query()
            wait_all(ckv_v, w_sem.at[CKV])

        during(i, t_attend, _B * per_group, b_attend)

        @pl.when(i == t_value - 1)
        def _():
            b_regroup_ctx()

        during(i, t_value, _H, b_value)

    def project_many(n, acc):
        return b_project(acc, [(0, 3 * n + u) for u in range(3)]
                         + [(1, 2 * n + u) for u in range(2)])

    def project_one(n, acc):
        p = jnp.where(n < 3, n % 2, 1)
        u = jnp.where(n < 3, 6 + n // 2 - 2 * p, n + 2)
        return b_project(acc, [(p, u)])

    assert _H // _NW == 8
    pl.loop(lag + 1, _H // _NW)(fetch_wob)
    out_b = lax.fori_loop(0, 2, project_many, jnp.zeros((_R, _PAD + _M), _F32))
    out_b = lax.fori_loop(0, 6, project_one, out_b)
    out = jnp.concatenate([outa_s[...], out_b[:, _PAD:]], axis=1)
    out_ref[...] = out[:_B].astype(out_ref.dtype)


def _scoped_kernel(*refs):
    pl.run_scoped(
        lambda *sems: _kernel(*refs, *sems),
        pltpu.SemaphoreType.DMA((2, _NBUF)),
        pltpu.SemaphoreType.DMA((8,)),
        pltpu.SemaphoreType.DMA((2, _H // _NW)),
    )


@jax.jit
def pallas_concat_heads__mha_block_cached__compressed_kv_cla__decode_kernel(
    A_x: jax.Array,
    A_k_cache: jax.Array,
    A_v_cache: jax.Array,
    A_wq: jax.Array,
    A_wo: jax.Array,
    B_x: jax.Array,
    B_c_kv: jax.Array,
    B_w_q: jax.Array,
    B_w_uk: jax.Array,
    B_w_uv: jax.Array,
    B_w_o: jax.Array,
):
    assert A_k_cache.shape == (_B, _H, _S, _D) and B_c_kv.shape == (_B, _S, _C)
    assert A_x.shape == (_B, 1, _M) and B_x.shape == (_B, 1, _M)

    operands = (
        A_x.reshape(_B, _M),
        A_k_cache.reshape(_B * _H, _S, _D),
        A_v_cache.reshape(_B * _H, _S, _D),
        A_wq.reshape(_NW, _M // _NW, _H * _D),
        A_wo.T.reshape(_NW, _M // _NW, _H * _D),
        B_x.reshape(_B, _M),
        B_c_kv.reshape(_NC, _B * _S // _NC, _C),
        B_w_q.reshape(_NW, _M * _H // _NW, _D),
        B_w_uk.reshape(_NW, _C * _H // _NW, _D),
        B_w_uv.reshape(_NW, _C * _H // _NW, _D),
        B_w_o.transpose(0, 2, 1).reshape(_NW, _H * _M // _NW, _D),
    )
    resident = [pltpu.VMEM(operands[i].shape, _BF) for i in (3, 4, 6, 7, 8, 9, 10)]
    out = pl.pallas_call(
        _scoped_kernel,
        out_shape=jax.ShapeDtypeStruct((_B, 2 * _M), A_x.dtype),
        in_specs=[pl.BlockSpec(memory_space=pltpu.HBM)] * len(operands),
        scratch_shapes=[
            pltpu.VMEM((_B, _M), _BF),
            pltpu.VMEM((_B, _M), _BF),
            pltpu.VMEM((_NBUF, _G, _TK, _D), _BF),
            pltpu.VMEM((_NBUF, _G, _TK, _D), _BF),
            *resident,
            pltpu.VMEM((_CW * _H // 2, _D), jnp.uint32),
            pltpu.VMEM((_H, _M, _D), _BF),
            pltpu.VMEM((_H, _C, _D), _BF),
            pltpu.VMEM((_H, _C, _D), _BF),
            pltpu.VMEM((_G * _R, _D), _F32),
            pltpu.VMEM((_B * _H // _G, _G, _D), _F32),
            pltpu.VMEM((_G, _D), _F32),
            pltpu.VMEM((_G, _D), _F32),
            pltpu.VMEM((_G, _D), _F32),
            pltpu.VMEM((_B * _G, _D), _F32),
            pltpu.VMEM((_R, _M), _F32),
            pltpu.VMEM((_C // _D, _H * _R, _D), _F32),
            pltpu.VMEM((_B, 2 * _H, _C), _BF),
            pltpu.VMEM((_H, _D), _F32),
            pltpu.VMEM((_H, _D), _F32),
            pltpu.VMEM((_H, _C), _F32),
            pltpu.VMEM((_C // _D, _B * _H, _D), _F32),
            pltpu.VMEM((_C // _D, _H * _R, _D), _F32),
            pltpu.VMEM((_H, _R, _D), _F32),
        ],
        compiler_params=pltpu.CompilerParams(vmem_limit_bytes=100 * 1024 * 1024),
    )(*operands)
    return out.reshape(_B, 1, 2 * _M)
```
